```python
import jax
import jax.numpy as jnp

def _softmax(x, axis=-1):
    return jax.nn.softmax(x, axis=axis)

def _gelu(x):
    return jax.nn.gelu(x, approximate=True)

def _silu(x):
    return jax.nn.silu(x)

def _sigmoid(x):
    return jax.nn.sigmoid(x)

def _layernorm(x, axis=-1, eps=1e-05):
    m = jnp.mean(x, axis=axis, keepdims=True)
    v = jnp.var(x, axis=axis, keepdims=True)
    return (x - m) / jnp.sqrt(v + eps)

def _scatter_add(tgt, idx, src, axis=0):
    return tgt.at[idx].add(src)

def _segment_sum(src, seg, n):
    return jax.ops.segment_sum(src, seg, n)

class _Rng:

    def __init__(self, key):
        self._k = key

    def _next(self):
        self._k, sub = jax.random.split(self._k)
        return sub

    def normal(self, shape):
        return jax.random.normal(self._next(), shape, dtype=jnp.bfloat16)

    def randint(self, lo, hi, shape):
        return jax.random.randint(self._next(), shape, lo, hi, dtype=jnp.int32)

    def uniform(self, shape, lo=0.0, hi=1.0):
        return jax.random.uniform(self._next(), shape, jnp.bfloat16, lo, hi)

    def permutation(self, n):
        return jax.random.permutation(self._next(), n)
kernel_name = 'adaLN_cond__sliding_block_cached__moe_arch_mod__prompt'

def setup_inputs():
    _rng = _Rng(jax.random.key(int.from_bytes(__import__("os").urandom(4), "little")))
    _w = lambda a: (lambda t: t.astype(jnp.bfloat16) if jnp.issubdtype(t.dtype, jnp.floating) else t)(jnp.asarray(a))

    def _A_setup():
        B, Sq, D = (1, 2048, 1024)
        Hq, Hkv, Sk, Dh = (32, 4, 2048, 128)
        assert Hq % Hkv == 0, (Hq, Hkv)
        return {'x': _w((lambda *s: _rng.normal(s) * 0.05)(B, Sq, D)), 'k_cache': _w((lambda *s: _rng.normal(s) * 0.05)(B, Hkv, Sk, Dh)), 'v_cache': _w((lambda *s: _rng.normal(s) * 0.05)(B, Hkv, Sk, Dh)), 'wq': _w((lambda *s: _rng.normal(s) * 0.05)(D, Hq * Dh) * D ** (-0.5)), 'wo': _w((lambda *s: _rng.normal(s) * 0.05)(Hq * Dh, D) * (Hq * Dh) ** (-0.5))}
    _A_in = _A_setup()

    def _B_setup():
        B, S, D, F, C = (1, 2048, 1024, 3584, 1)
        return {'x': _w((lambda *s: _rng.normal(s) * 0.05)(B, S, D)), 'w_r': _w((lambda *s: _rng.normal(s) * 0.05)(D)), 'w_gate': _w((lambda *s: _rng.normal(s) * 0.05)(D, F)), 'w_up': _w((lambda *s: _rng.normal(s) * 0.05)(D, F)), 'w_down': _w((lambda *s: _rng.normal(s) * 0.05)(F, D))}
    _B_in = _B_setup()
    return {'A_x': _A_in['x'], 'A_k_cache': _A_in['k_cache'], 'A_v_cache': _A_in['v_cache'], 'A_wq': _A_in['wq'], 'A_wo': _A_in['wo'], 'B_x': _B_in['x'], 'B_w_r': _B_in['w_r'], 'B_w_gate': _B_in['w_gate'], 'B_w_up': _B_in['w_up'], 'B_w_down': _B_in['w_down'], 'c': _w((lambda *s: _rng.normal(s) * 0.05)(1, 1024)), 'w_mod': _w((lambda *s: _rng.normal(s) * 0.05)(1024, 6 * 1024) * 1024 ** (-0.5))}

def reference(A_x, A_k_cache, A_v_cache, A_wq, A_wo, B_x, B_w_r, B_w_gate, B_w_up, B_w_down, c, w_mod):

    def _A_ref(x, k_cache, v_cache, wq, wo):
        B, Sq, D = x.shape
        Hq, Dh = (32, 128)
        Hkv, Sk = (k_cache.shape[1], k_cache.shape[2])
        W = min(4096, max(256, Sk // 4))
        rep = Hq // Hkv
        q = (lambda x, *d: x.transpose(*d))((x @ wq).reshape(B, Sq, Hq, Dh), 0, 2, 1, 3)
        k = jnp.repeat(k_cache[:, :, Sk - W:, :], rep, axis=1)
        v = jnp.repeat(v_cache[:, :, Sk - W:, :], rep, axis=1)
        scores = jnp.einsum('bhqd,bhkd->bhqk', q, k) * Dh ** (-0.5)
        p = _softmax(scores, axis=-1)
        o = jnp.einsum('bhqk,bhkd->bhqd', p, v)
        return (lambda x, *d: x.transpose(*d))(o, 0, 2, 1, 3).reshape(B, Sq, Hq * Dh) @ wo

    def _B_ref(x, w_r, w_gate, w_up, w_down):
        B, S, D = x.shape
        C = 1
        r = x @ w_r
        idx = jnp.argsort(-r, axis=-1)[:, :C]
        idx_e = jnp.repeat(idx.reshape(B, C, 1), D, axis=2)
        x_sel = jnp.take_along_axis(x, idx_e, axis=1)
        g = _silu(x_sel @ w_gate)
        u = x_sel @ w_up
        y = g * u @ w_down
        r_sel = _sigmoid(jnp.take_along_axis(r, idx, axis=1))
        y = y * r_sel.reshape(B, C, 1)
        b_off = (jnp.arange(B) * S).reshape(B, 1)
        flat_idx = (idx + b_off).reshape(B * C)
        zero = (x * 0.0).reshape(B * S, D)
        upd = _scatter_add(zero, flat_idx, y.reshape(B * C, D), axis=0)
        return x + upd.reshape(B, S, D)
    x = A_x
    mod = (_silu(c) @ w_mod).reshape(c.shape[0], 6, 1, -1)
    sa, ca, ga, sb, cb, gb = (mod[:, 0].copy(), mod[:, 1].copy(), mod[:, 2].copy(), mod[:, 3].copy(), mod[:, 4].copy(), mod[:, 5].copy())
    h = _layernorm(x, axis=-1) * (1 + ca) + sa
    x = x + ga * _A_ref(h, A_k_cache, A_v_cache, A_wq, A_wo)
    h = _layernorm(x, axis=-1) * (1 + cb) + sb
    x = x + gb * _B_ref(h, B_w_r, B_w_gate, B_w_up, B_w_down)
    return x
```

```python
import functools
import jax
import jax.numpy as jnp
import numpy as np
import jax.experimental.pallas as pl
import jax.experimental.pallas.tpu as pltpu

S, D, HQ, HKV, DH, SK, W, F = 2048, 1024, 32, 4, 128, 2048, 512, 3584
REP = HQ // HKV
LOG2E = 1.4426950408889634
SCALE = DH ** -0.5
EPS = 1e-5
bf16 = jnp.bfloat16
f32 = jnp.float32
NT = (((1,), (1,)), ((), ()))


def _ln(xf):
    m = jnp.mean(xf, axis=-1, keepdims=True)
    xc = xf - m
    v = jnp.mean(xc * xc, axis=-1, keepdims=True)
    return xc * jax.lax.rsqrt(v + EPS)


def _dot(a, b):
    return jnp.dot(a, b, preferred_element_type=f32)


def make(CH=16, LNP=(0, 1, 2, 3), EPP=(4, 5, 6, 7), WHERE='after_o', NIT=None, TAIL=True, MODC=4, LNPOS=5, EPIPOS=0, flags=None, DRAIN_SPLIT=4, RCP="nr"):
    TM = 256
    NB = S // TM
    NDT = D // 128
    NFT = F // 128
    TQ = TM // 4
    NITEMS = NB * HKV

    def kernel(x_hbm, k_hbm, v_hbm, wq_hbm, wo_hbm, wr_ref, wg_hbm, wu_hbm, wd_hbm, c_ref, wmod_hbm,
               out_hbm,
               x_buf, k_buf, v_buf, wq_buf, wo_buf, wg_buf, wu_buf, wd_buf, wmod_buf, mod_buf,
               h_buf, o_buf, att_buf, out_buf, best_v, best_i, sems):
        si = [0]
        def new_sem(n=1):
            i = si[0]; si[0] += n
            return i
        s_mod0 = new_sem(MODC); s_mod = new_sem(); s_x0 = new_sem(); s_x1 = new_sem(); s_xr = new_sem()
        s_wq0 = new_sem(2); s_item = new_sem(4)
        s_wg = new_sem(); s_wu = new_sem(); s_wd = new_sem(); s_out = new_sem(); s_fin = new_sem()

        MR = D // MODC
        def cp_wmod0(i):
            return pltpu.make_async_copy(wmod_hbm.at[pl.ds(i * MR, MR), pl.ds(0, 2048)], wmod_buf.at[0, pl.ds(i * MR, MR)], sems.at[s_mod0 + i])
        def cp_wmod(a):
            return pltpu.make_async_copy(wmod_hbm.at[:, pl.ds(a * 2048, 2048)], wmod_buf.at[a], sems.at[s_mod])
        cp_x0 = pltpu.make_async_copy(x_hbm.at[pl.ds(0, TM)], x_buf.at[pl.ds(0, TM)], sems.at[s_x0])
        cp_x1 = pltpu.make_async_copy(x_hbm.at[pl.ds(TM, TM)], x_buf.at[pl.ds(TM, TM)], sems.at[s_x1])
        cp_xr = pltpu.make_async_copy(x_hbm.at[pl.ds(2 * TM, S - 2 * TM)], x_buf.at[pl.ds(2 * TM, S - 2 * TM)], sems.at[s_xr])
        def cp_wq(t, sem):
            return pltpu.make_async_copy(wq_hbm.at[:, pl.ds(t * 128, 128)], wq_buf.at[t], sems.at[sem])
        def cp_wo(g, n, sem):
            return pltpu.make_async_copy(wo_hbm.at[pl.ds(g * 1024, 1024), pl.ds(n * 128, 128)], wo_buf.at[g, n], sems.at[sem])
        def cp_k(g, sem):
            return pltpu.make_async_copy(k_hbm.at[g, pl.ds(SK - W, W), :], k_buf.at[g], sems.at[sem])
        def cp_v(g, sem):
            return pltpu.make_async_copy(v_hbm.at[g, pl.ds(SK - W, W), :], v_buf.at[g], sems.at[sem])
        def item_copies(g):
            sem = s_item + g
            cps = [cp_k(g, sem), cp_v(g, sem)]
            cps += [cp_wq(t, sem) for t in range(8 * g, 8 * g + 8)]
            if g > 0:
                cps += [cp_wo(g - 1, n, sem) for n in range(NDT)]
            return cps
        def cp_wg(n):
            return pltpu.make_async_copy(wg_hbm.at[:, pl.ds(pl.multiple_of(n * 128, 128), 128)], wg_buf.at[n], sems.at[s_wg])
        def cp_wu(n):
            return pltpu.make_async_copy(wu_hbm.at[:, pl.ds(pl.multiple_of(n * 128, 128), 128)], wu_buf.at[n], sems.at[s_wu])
        def cp_wd(n):
            return pltpu.make_async_copy(wd_hbm.at[:, pl.ds(pl.multiple_of(n * 128, 128), 128)], wd_buf.at[n], sems.at[s_wd])
        def cp_out(e):
            r0 = pl.multiple_of(e * TQ, TQ)
            return pltpu.make_async_copy(out_buf.at[pl.ds(r0, TQ)], out_hbm.at[pl.ds(r0, TQ)], sems.at[s_out])

        cp_x0.start()
        for i in range(MODC):
            cp_wmod0(i).start()
        for c_ in item_copies(0): c_.start()
        cp_x1.start()
        for c_ in item_copies(1): c_.start()

        cf = c_ref[...].astype(f32)
        sc = (cf * jax.nn.sigmoid(cf)).astype(bf16)
        sc8 = jnp.broadcast_to(sc, (8, D))

        def modrow(i):
            return mod_buf[i][0:1, :]

        def ln1_rows(xv, nrows, hpar, hr0):
            xf = xv.astype(f32)
            h = (_ln(xf) * (1.0 + modrow(1)) + modrow(0)).astype(bf16)
            for c in range(NDT):
                h_buf[hpar, c, pl.ds(hr0, nrows), :] = h[:, c * 128:(c + 1) * 128]

        def load_h(hpar):
            return jnp.concatenate([h_buf[hpar, c] for c in range(NDT)], axis=1)

        def qproj(t, hv):
            q = _dot(hv, wq_buf[t])
            return (q * (SCALE * LOG2E)).astype(bf16)

        def qk(g, qh):
            return jax.lax.dot_general(qh, k_buf[g], NT, preferred_element_type=f32)

        def softmax(s):
            m = jnp.max(s, axis=-1, keepdims=True)
            p = jnp.exp2(s - m)
            l = jnp.sum(p, axis=-1, keepdims=True)
            if RCP == "nr":
                r = pl.reciprocal(l, approx=True)
                r = r * (2.0 - l * r)
            elif RCP == "approx":
                r = pl.reciprocal(l, approx=True)
            else:
                r = 1.0 / l
            return p.astype(bf16), r

        def pv(g, p, r):
            o = _dot(p, v_buf[g])
            return (o * r).astype(bf16)

        def load_o(opar, r0=0, nrows=TM):
            return jnp.concatenate([o_buf[opar, j, pl.ds(r0, nrows), :] for j in range(REP)], axis=1)

        def epilogue(r0, nrows, att, xv):
            xf = xv.astype(f32)
            x1 = (xf + modrow(2) * att).astype(bf16)
            x_buf[pl.ds(r0, nrows), :] = x1
            x1f = x1.astype(f32)
            h2 = (_ln(x1f) * (1.0 + modrow(4)) + modrow(3)).astype(bf16).astype(f32)
            wr = wr_ref[...].astype(f32).reshape(1, D)
            r = jnp.sum(h2 * wr, axis=-1, keepdims=True)
            out_buf[pl.ds(r0, nrows), :] = (x1f + modrow(5) * (h2 + h2 * 0.0)).astype(bf16)
            return r

        def track(r0, r, valid):
            rid = r0 + jax.lax.broadcasted_iota(jnp.int32, (CH, 1), 0)
            bv = best_v[...]
            upd = r > bv
            if valid is not None:
                upd = jnp.logical_and(upd, valid)
            best_i[...] = jnp.where(upd, rid, best_i[...])
            best_v[...] = jnp.where(upd, r, bv)

        o_buf[1] = jnp.zeros(o_buf.shape[1:], bf16)
        wo_buf[4] = jnp.zeros(wo_buf.shape[1:], bf16)
        att_buf[...] = jnp.zeros(att_buf.shape, f32)
        x_buf[pl.ds(S, TQ), :] = jnp.zeros((TQ, D), bf16)
        mod_buf[...] = jnp.zeros(mod_buf.shape, f32)
        best_v[...] = jnp.full(best_v.shape, -jnp.inf, f32)
        best_i[...] = jnp.zeros(best_i.shape, jnp.int32)

        m = None
        for i in range(MODC):
            cp_wmod0(i).wait()
            d = _dot(sc8[:, i * MR:(i + 1) * MR], wmod_buf[0, i * MR:(i + 1) * MR, :])
            m = d if m is None else m + d
        m = m.astype(bf16).astype(f32)
        mod_buf[0] = m[:, :D]
        mod_buf[1] = m[:, D:]
        cp_x0.wait()
        ln1_rows(x_buf[pl.ds(0, TM), :], TM, 0, 0)

        def item(i, carry):
            b = i // 4
            g = i % 4
            opar = i % 2
            gp = (i + 3) % 4
            apar = ((i + 3) // 4 + 1) % 2
            wslot = jnp.where(i == 0, 4, gp)
            hpar = b % 2

            @pl.when(i < 12)
            def _():
                @pl.when(i == 0)
                def _():
                    cp_x1.wait()
                    for c_ in item_copies(0): c_.wait()
                    for c_ in item_copies(2): c_.start()
                @pl.when(i == 1)
                def _():
                    for c_ in item_copies(1): c_.wait()
                    for c_ in item_copies(3): c_.start()
                @pl.when(i == 2)
                def _():
                    for c_ in item_copies(2): c_.wait()
                    for n in range(NDT): cp_wo(3, n, s_xr).start()
                    cp_xr.start()
                    cp_wmod(1).start(); cp_wmod(2).start()
                @pl.when(i == 3)
                def _():
                    for c_ in item_copies(3): c_.wait()
                @pl.when(i == 4)
                def _():
                    for n in range(NDT): cp_wo(3, n, s_xr).wait()
                    cp_xr.wait()
                    cp_wmod(1).wait(); cp_wmod(2).wait()
                    for a in (1, 2):
                        mm = _dot(sc8, wmod_buf[a]).astype(bf16).astype(f32)
                        mod_buf[2 * a] = mm[:, :D]
                        mod_buf[2 * a + 1] = mm[:, D:]
                @pl.when(jnp.logical_and(i >= 4, i < 11))
                def _():
                    j = i - 4
                    for u in range(4):
                        cp_wg(4 * j + u).start()
                        cp_wu(4 * j + u).start()
                @pl.when(i >= 4)
                def _():
                    cp_wd(i - 4).start()
            @pl.when(i >= 6)
            def _():
                cp_out(i - 6).start()

            NCH = TQ // CH
            e = i - 5
            valid = e >= 0
            er0 = pl.multiple_of(jnp.where(valid, e, NB * 4) * TQ, TQ)
            ec = jnp.maximum(e, 0)
            epar = (ec // 4) % 2
            ea0 = pl.multiple_of((ec % 4) * TQ, TQ)
            bn = jnp.minimum(b + 1, NB - 1)
            lr0 = pl.multiple_of(bn * TM + g * TQ, TQ)

            hv = load_h(hpar)
            og = load_o(1 - opar)
            xl = x_buf[pl.ds(lr0, TQ), :]
            xe = x_buf[pl.ds(er0, TQ), :]
            ae = att_buf[epar, pl.ds(ea0, TQ), :]

            def do_ln(u):
                ln1_rows(xl[u * CH:(u + 1) * CH], CH, (b + 1) % 2, pl.multiple_of(g * TQ + u * CH, CH))

            def do_epi(u):
                r0 = pl.multiple_of(er0 + u * CH, CH)
                r = epilogue(r0, CH, ae[u * CH:(u + 1) * CH], xe[u * CH:(u + 1) * CH])
                track(r0, r, valid)

            t0 = g * REP
            qs = {0: qproj(t0, hv), 1: qproj(t0 + 1, hv)}
            ss = {0: qk(g, qs.pop(0))}
            for j in range(REP):
                if j + 1 < REP:
                    ss[j + 1] = qk(g, qs.pop(j + 1))
                if j + 2 < REP:
                    qs[j + 2] = qproj(t0 + j + 2, hv)
                c = _dot(og, wo_buf[wslot, j])
                old = att_buf[apar, :, j * 128:(j + 1) * 128]
                att_buf[apar, :, j * 128:(j + 1) * 128] = jnp.where(gp == 0, 0.0, old) + c
                def extra():
                    for u in range(NCH):
                        if LNP[u] == j:
                            do_ln(u)
                        if EPP[u] == j:
                            do_epi(u)
                if WHERE == 'after_o':
                    extra()
                p, r = softmax(ss.pop(j))
                o_buf[opar, j] = pv(g, p, r)
                if WHERE == 'after_pv':
                    extra()
            return carry

        NI = NIT or NITEMS
        jax.lax.fori_loop(0, NI, item, 0)

        if NI < NITEMS or not TAIL:
            for e in range(max(NI - 6, 0), NB * 4):
                cp_out(e).start()
            pltpu.make_async_copy(out_buf.at[pl.ds(0, S)], out_hbm, sems.at[s_out]).wait()
            assert NI >= 12
            pltpu.make_async_copy(wg_buf, wg_buf, sems.at[s_wg]).wait()
            pltpu.make_async_copy(wu_buf, wu_buf, sems.at[s_wu]).wait()
            pltpu.make_async_copy(wd_buf, wd_buf, sems.at[s_wd]).wait()
            return

        cp_out(26).start()
        def epi_static(e, att):
            for u in range(TQ // CH):
                r0 = e * TQ + u * CH
                r = epilogue(r0, CH, att(u), x_buf[pl.ds(r0, CH), :])
                track(r0, r, None)
            cp_out(e).start()
        epi_static(27, lambda u: att_buf[0, pl.ds(3 * TQ + u * CH, CH), :])
        DS = DRAIN_SPLIT
        RS = TM // DS
        opar_last = (NITEMS - 1) % 2
        for u in range(DS):
            og = load_o(opar_last, u * RS, RS)
            for n in range(NDT):
                c = _dot(og, wo_buf[3, n])
                att_buf[1, pl.ds(u * RS, RS), n * 128:(n + 1) * 128] += c
            for qq in range(u * 4 // DS, (u + 1) * 4 // DS):
                epi_static(28 + qq, lambda u, qq=qq: att_buf[1, pl.ds(qq * TQ + u * CH, CH), :])

        bv = best_v[...]
        mx = jnp.max(bv)
        idx = jnp.min(jnp.where(bv == mx, best_i[...], S))
        idx = jnp.clip(idx, 0, S - 1)
        base = pl.multiple_of((idx // 16) * 16, 16)
        x1f = x_buf[pl.ds(base, 16), :].astype(f32)
        h2b = (_ln(x1f) * (1.0 + modrow(4)) + modrow(3)).astype(bf16)
        h2 = h2b.astype(f32)
        pltpu.make_async_copy(wg_buf, wg_buf, sems.at[s_wg]).wait()
        pltpu.make_async_copy(wu_buf, wu_buf, sems.at[s_wu]).wait()
        pltpu.make_async_copy(wd_buf, wd_buf, sems.at[s_wd]).wait()
        acts = []
        for n in range(NFT):
            g_ = _dot(h2b, wg_buf[n])
            u_ = _dot(h2b, wu_buf[n])
            acts.append((g_ * jax.nn.sigmoid(g_) * u_).astype(bf16))
        a_ = jnp.concatenate(acts, axis=1)
        y = jnp.concatenate([_dot(a_, wd_buf[n]) for n in range(NDT)], axis=1)
        y = y * jax.nn.sigmoid(jnp.full((1, 1), mx, f32))
        rid = base + jax.lax.broadcasted_iota(jnp.int32, (16, 1), 0)
        upd = jnp.where(rid == idx, y, h2 * 0.0)
        pltpu.make_async_copy(out_buf.at[pl.ds(0, S)], out_hbm, sems.at[s_out]).wait()
        out_buf[pl.ds(base, 16), :] = (x1f + modrow(5) * (h2 + upd)).astype(bf16)
        fin = pltpu.make_async_copy(out_buf.at[pl.ds(base, 16)], out_hbm.at[pl.ds(base, 16)], sems.at[s_fin])
        fin.start()
        fin.wait()

    NSEM = MODC + 4 + 2 + 4 + 5

    def fn(A_x, A_k_cache, A_v_cache, A_wq, A_wo, B_x, B_w_r, B_w_gate, B_w_up, B_w_down, c, w_mod):
        x2 = A_x.reshape(S, D)
        k3 = A_k_cache.reshape(HKV, SK, DH)
        v3 = A_v_cache.reshape(HKV, SK, DH)
        hbm = pl.BlockSpec(memory_space=pl.ANY)
        vm = pl.BlockSpec(memory_space=pltpu.VMEM)
        out = pl.pallas_call(
            kernel,
            out_shape=jax.ShapeDtypeStruct((S, D), bf16),
            in_specs=[hbm, hbm, hbm, hbm, hbm, vm, hbm, hbm, hbm, vm, hbm],
            out_specs=hbm,
            scratch_shapes=[
                pltpu.VMEM((S + TQ, D), bf16),
                pltpu.VMEM((HKV, W, DH), bf16),
                pltpu.VMEM((HKV, W, DH), bf16),
                pltpu.VMEM((HQ, D, 128), bf16),
                pltpu.VMEM((HKV + 1, NDT, 1024, 128), bf16),
                pltpu.VMEM((NFT, D, 128), bf16),
                pltpu.VMEM((NFT, D, 128), bf16),
                pltpu.VMEM((NDT, F, 128), bf16),
                pltpu.VMEM((3, D, 2048), bf16),
                pltpu.VMEM((6, 8, D), f32),
                pltpu.VMEM((2, NDT, TM, 128), bf16),
                pltpu.VMEM((2, REP, TM, 128), bf16),
                pltpu.VMEM((2, TM, D), f32),
                pltpu.VMEM((S + TQ, D), bf16),
                pltpu.VMEM((CH, 1), f32),
                pltpu.VMEM((CH, 1), jnp.int32),
                pltpu.SemaphoreType.DMA((NSEM,)),
            ],
            compiler_params=pltpu.CompilerParams(vmem_limit_bytes=126 * 1024 * 1024, flags=flags),
        )(x2, k3, v3, A_wq, A_wo, B_w_r, B_w_gate, B_w_up, B_w_down, c, w_mod)
        return out.reshape(1, S, D)

    return jax.jit(fn)


_impl = make()


@jax.jit
def pallas_adaLN_cond__sliding_block_cached__moe_arch_mod__prompt_kernel(
    A_x, A_k_cache, A_v_cache, A_wq, A_wo, B_x, B_w_r, B_w_gate, B_w_up, B_w_down, c, w_mod,
):
    return _impl(A_x, A_k_cache, A_v_cache, A_wq, A_wo, B_x, B_w_r, B_w_gate, B_w_up, B_w_down, c, w_mod)
```

```python
import contextlib

import jax
import jax.numpy as jnp
import jax.experimental.pallas as pl
import jax.experimental.pallas.tpu as pltpu

S, D, HQ, HKV, DH, SK, W, F = 2048, 1024, 32, 4, 128, 2048, 512, 3584
REP = HQ // HKV
LOG2E = 1.4426950408889634
SCALE = DH ** -0.5
EPS = 1e-5
bf16 = jnp.bfloat16
f32 = jnp.float32
i32 = jnp.int32
NT = (((1,), (1,)), ((), ()))

TM = 256
NB = S // TM
NDT = D // 128
NFT = F // 128
TQ = TM // 4
NQ = S // TQ
NITEMS = NB * HKV


def _ln(xf):
    m = jnp.mean(xf, axis=-1, keepdims=True)
    xc = xf - m
    v = jnp.mean(xc * xc, axis=-1, keepdims=True)
    return xc * jax.lax.rsqrt(v + EPS)


def _dot(a, b):
    return jnp.dot(a, b, preferred_element_type=f32)


def _shr(x, n):
    return x >> n if isinstance(x, int) else jax.lax.shift_right_logical(x, n)


def _and(x, n):
    return x & n


def _mult(x, n):
    return x if isinstance(x, int) else pl.multiple_of(x, n)


def make(ORDER='A', SPLIT=False, DPER=1, H2BUF=True, PADW=128, SCOPES=False, CH=16, LNP=(0, 1, 2, 3), EPP=(4, 5, 6, 7), MODC=4, DRAIN_SPLIT=4, flags=None,
         WQW=((0, 1), (1, 2), (2, 3), (3, 5), (5, 8)), TAIL=True):
    NCH = TQ // CH

    def kernel(x_hbm, k_hbm, v_hbm, wq_hbm, wo_hbm, wr_hbm, wg_hbm, wu_hbm, wd_hbm, c_hbm, wmod_hbm,
               out_hbm,
               x_buf, k_buf, v_buf, wq_buf, wo_buf, wg_buf, wu_buf, wd_buf, wmod_buf, mod_buf,
               h_buf, o_buf, att_buf, out_buf, h2_buf, best_v, best_i, c_ref, wr_ref, sems):
        nsem = [0]

        def new_sem():
            nsem[0] += 1
            return nsem[0] - 1

        def scope(name):
            return jax.named_scope(name) if SCOPES else contextlib.nullcontext()

        def copy(src, dst, sem):
            return pltpu.make_async_copy(src, dst, sems.at[sem])

        class Group:
            def __init__(self, fn):
                self.sem = new_sem()
                self.cps = fn(self.sem)

            def start(self):
                for c_ in self.cps:
                    c_.start()

            def wait(self):
                for c_ in self.cps:
                    c_.wait()

        def wld(ref, *idx):
            return pltpu.bitcast(ref.bitcast(jnp.uint32)[idx], bf16)

        def g_x(r0, r1):
            return Group(lambda s: [copy(x_hbm.at[pl.ds(r0, r1 - r0)], x_buf.at[pl.ds(r0, r1 - r0)], s)])

        def g_wq(t0, t1):
            return Group(lambda s: [copy(wq_hbm.at[:, pl.ds(t * 128, 128)], wq_buf.at[t], s) for t in range(t0, t1)])

        def g_wo(g):
            return Group(lambda s: [copy(wo_hbm.at[pl.ds(g * 1024, 1024), pl.ds(n * 128, 128)], wo_buf.at[g, n], s)
                                    for n in range(NDT)])

        def g_k(g):
            return Group(lambda s: [copy(k_hbm.at[g, pl.ds(SK - W, W), :], k_buf.at[g], s)])

        def g_v(g):
            return Group(lambda s: [copy(v_hbm.at[g, pl.ds(SK - W, W), :], v_buf.at[g], s)])

        def g_wmod(c0, c1):
            return Group(lambda s: [copy(wmod_hbm.at[:, pl.ds(c0, c1 - c0)], wmod_buf.at[:, pl.ds(c0, c1 - c0)], s)])

        G_c = Group(lambda s: [copy(c_hbm, c_ref, s)])
        G_wr = Group(lambda s: [copy(wr_hbm, wr_ref, s)])
        G_x0, G_x1 = g_x(0, TM), g_x(TM, 2 * TM)
        G_xa, G_xb, G_xc = g_x(2 * TM, 2 * TM + TQ), g_x(2 * TM + TQ, 4 * TM), g_x(4 * TM, S)
        G_mod0 = [g_wmod(i * 2048 // MODC, (i + 1) * 2048 // MODC) for i in range(MODC)]
        G_mod12 = g_wmod(2048, 6144)
        G_wq0 = [g_wq(a, b) for a, b in WQW]
        G_wq = [None] + [g_wq(8 * g, 8 * g + 8) for g in range(1, HKV)]
        G_k = [g_k(g) for g in range(HKV)]
        G_v = [g_v(g) for g in range(HKV)]
        G_wo = [g_wo(g) for g in range(HKV)]
        G_ffn = Group(lambda s: [copy(wg_hbm, wg_buf, s), copy(wu_hbm, wu_buf, s), copy(wd_hbm, wd_buf.at[:, pl.ds(0, D)], s)])
        s_out = new_sem()
        s_fin = new_sem()
        assert nsem[0] <= NSEM

        def cp_out(e):
            r0 = _mult(e * TQ, TQ)
            return copy(out_buf.at[pl.ds(r0, TQ)], out_hbm.at[pl.ds(r0, TQ)], s_out)

        first_order = [G_c, G_x0] + G_mod0 + [G_wq0[0], G_wq0[1], G_k[0], G_v[0]] + G_wq0[2:] + [G_x1, G_wr]
        first_order += [G_wo[0], G_xa, G_wq[1], G_k[1], G_v[1], G_xb, G_wo[1], G_wq[2], G_k[2], G_v[2], G_wo[2]]
        later_order = [G_wq[3], G_k[3], G_v[3], G_wo[3], G_mod12, G_xc, G_ffn]
        for grp in first_order:
            grp.start()

        def modrow(i):
            return mod_buf[i][0:1, :]

        def normalize(xv):
            return _ln(xv.astype(f32))

        def store_h(hn, slot, hr0, nrows):
            h = (hn * (1.0 + modrow(1)) + modrow(0)).astype(bf16)
            for c in range(NDT):
                h_buf[slot, c, pl.ds(hr0, nrows), :] = h[:, c * 128:(c + 1) * 128]

        def load_h(slot):
            return jnp.concatenate([h_buf[slot, c] for c in range(NDT)], axis=1)

        def qproj(t, hv):
            q = _dot(hv, wld(wq_buf, t))
            return (q * (SCALE * LOG2E)).astype(bf16)

        def qk(g, qh):
            return jax.lax.dot_general(qh, wld(k_buf, g), NT, preferred_element_type=f32)

        def softmax(s):
            m = jnp.max(s, axis=-1, keepdims=True)
            p = jnp.exp2(s - m)
            l = jnp.sum(p, axis=-1, keepdims=True)
            r = pl.reciprocal(l, approx=True)
            r = r * (2.0 - l * r)
            return p.astype(bf16), r

        def pv(g, p, r):
            return (_dot(p, wld(v_buf, g)) * r).astype(bf16)

        def load_o(slot, r0=0, nrows=TM):
            return jnp.concatenate([o_buf[slot, j, pl.ds(r0, nrows), :] for j in range(REP)], axis=1)

        def epilogue(r0, att, xv):
            x1 = (xv.astype(f32) + modrow(2) * att).astype(bf16)
            x_buf[pl.ds(r0, CH), :] = x1
            x1f = x1.astype(f32)
            h2b_ = (_ln(x1f) * (1.0 + modrow(4)) + modrow(3)).astype(bf16)
            if H2BUF:
                h2_buf[pl.ds(r0, CH), :] = h2b_
            h2 = h2b_.astype(f32)
            wr = wr_ref[...].astype(f32).reshape(1, D)
            r = jnp.sum(h2 * wr, axis=-1, keepdims=True)
            out_buf[pl.ds(r0, CH), :] = (x1f + modrow(5) * (h2 + h2 * 0.0)).astype(bf16)
            return r

        def track(r0, r, valid):
            rid = r0 + jax.lax.broadcasted_iota(i32, (CH, 1), 0)
            bv = best_v[...]
            upd = r > bv
            if valid is not None:
                upd = jnp.logical_and(upd, valid)
            best_i[...] = jnp.where(upd, rid, best_i[...])
            best_v[...] = jnp.where(upd, r, bv)

        def mod_tiles(sc8, n0, n1):
            for n in range(n0, n1):
                d = _dot(sc8, wmod_buf[:, n * 128:(n + 1) * 128]).astype(bf16).astype(f32)
                mod_buf[n // 8, :, (n % 8) * 128:(n % 8 + 1) * 128] = d

        att_buf[...] = jnp.zeros(att_buf.shape, f32)
        x_buf[pl.ds(S, TQ), :] = jnp.zeros((TQ, D), bf16)
        mod_buf[...] = jnp.zeros(mod_buf.shape, f32)
        best_v[...] = jnp.full(best_v.shape, -jnp.inf, f32)
        best_i[...] = jnp.zeros(best_i.shape, i32)

        G_c.wait()
        cf = c_ref[...].astype(f32)
        sc8 = jnp.broadcast_to((cf * jax.nn.sigmoid(cf)).astype(bf16), (8, D))
        with scope("p_ln0a"):
            G_x0.wait()
            hn0 = normalize(x_buf[pl.ds(0, TM), :])
        with scope("p_mod0"):
            for i in range(MODC):
                G_mod0[i].wait()
                mod_tiles(sc8, i * 16 // MODC, (i + 1) * 16 // MODC)
        with scope("p_ln0b"):
            store_h(hn0, 0, 0, TM)

        def item(i, first, steady=False):
            par = _and(i, 1)
            g = _and(_shr(i, 1), 3)
            pair = _shr(i, 3)
            rb0 = pair * (2 * TM) + par * TM
            hslot = _and(pair, 1) * 2 + par
            ip = i - 1
            gp = _and(_shr(ip, 1), 3)
            aslot = _and(_shr(ip, 3), 1) * 2 + _and(ip, 1)
            if not first:
                u_ln = _and(ip, 7)
                pn = _shr(ip, 3) + 1
                lr0 = _mult(jnp.minimum(pn * 8 + u_ln, NQ - 1) * TQ, TQ)
                lslot = _and(pn, 1) * 2 + _shr(u_ln, 2)
                lh0 = _and(u_ln, 3) * TQ
                e = i - 8
                valid = e >= 0
                ec = jnp.maximum(e, 0)
                er0 = _mult(jnp.where(valid, e, NQ) * TQ, TQ)
                eslot = _and(_shr(ec, 2), 3)
                ea0 = _mult(_and(ec, 3) * TQ, TQ)

            if steady:
                cp_out(e - 1).start()
            elif not first:
                with scope('top'):
                    @pl.when(i < 9)
                    def _():
                        for k_, grps in ((1, [G_wo[0], G_xa, G_wr]), (2, [G_wq[1], G_k[1], G_v[1], G_xb]), (3, [G_wo[1]]),
                                         (4, [G_wq[2], G_k[2], G_v[2]]), (5, [G_wo[2]]), (6, [G_wq[3], G_k[3], G_v[3]]),
                                         (7, [G_wo[3], G_mod12]), (8, [G_xc])):
                            @pl.when(i == k_)
                            def _():
                                for grp in grps:
                                    grp.wait()
                                if k_ == 7:
                                    mod_tiles(sc8, 16, 48)

                    @pl.when(i >= 9)
                    def _():
                        cp_out(e - 1).start()

            with scope('item'):
                hv = load_h(hslot)
                if not first:
                    og = load_o(1 - par)
                    xl = x_buf[pl.ds(lr0, TQ), :]
                    xe = x_buf[pl.ds(er0, TQ), :]
                    ae = att_buf[eslot, pl.ds(ea0, TQ), :]

                def do_ln(u):
                    store_h(normalize(xl[u * CH:(u + 1) * CH]), lslot, _mult(lh0 + u * CH, CH), CH)

                def do_epi(u):
                    r0 = _mult(er0 + u * CH, CH)
                    r = epilogue(r0, ae[u * CH:(u + 1) * CH], xe[u * CH:(u + 1) * CH])
                    track(r0, r, valid)

                def need_wq(t):
                    if first:
                        for grp, (a, _) in zip(G_wq0, WQW):
                            if a == t:
                                grp.wait()

                def qp(j):
                    need_wq(j)
                    return qproj(g * REP + j, hv)

                qs = {0: qp(0), 1: qp(1)}
                if first:
                    G_k[0].wait()
                ss = {0: qk(g, qs.pop(0))}
                for j in range(REP):
                    def f_qk():
                        if j + 1 < REP:
                            ss[j + 1] = qk(g, qs.pop(j + 1))

                    def f_q():
                        if j + 2 < REP:
                            qs[j + 2] = qp(j + 2)

                    def f_o():
                        if not first:
                            c = _dot(og, wld(wo_buf, gp, j))
                            old = att_buf[aslot, :, j * 128:(j + 1) * 128]
                            att_buf[aslot, :, j * 128:(j + 1) * 128] = jnp.where(gp == 0, 0.0, old) + c

                    def f_x():
                        if not first:
                            for u in range(NCH):
                                if LNP[u] == j:
                                    do_ln(u)
                                if EPP[u] == j:
                                    do_epi(u)
                        else:
                            if j == 1:
                                for grp in later_order:
                                    grp.start()
                            if j == 4:
                                G_x1.wait()
                            if j >= 4:
                                r0 = (j - 4) * TQ
                                store_h(normalize(x_buf[pl.ds(TM + r0, TQ), :]), 1, r0, TQ)

                    pr = {}

                    def f_sm():
                        pr[0] = softmax(ss.pop(j))

                    def f_pv():
                        if first and j == 0:
                            G_v[0].wait()
                        o_buf[par, j] = pv(g, *pr[0])

                    tbl = dict(q=f_q, k=f_qk, o=f_o, x=f_x, s=f_sm, p=f_pv)
                    seq = dict(A="kqoxsp", B="skqoxp", C="koqxsp", D="qksopx", E="kqsoxp", F="kqospx", G="kxqosp", H="kqsxop")[ORDER]
                    for ch_ in seq:
                        tbl[ch_]()

        item(0, True)

        def loop_body(i, carry):
            item(i, False)
            return carry
        if SPLIT:
            jax.lax.fori_loop(1, 9, loop_body, 0)

            def loop_body2(i, carry):
                item(i, False, True)
                return carry
            jax.lax.fori_loop(9, NITEMS, loop_body2, 0)
        else:
            jax.lax.fori_loop(1, NITEMS, loop_body, 0)

        with scope('drain'):
            cp_out(NQ - 9).start()

            DS = DRAIN_SPLIT
            RS = TM // DS
            def chunk(e, u, slot):
                r0 = e * TQ + u * CH
                r = epilogue(r0, att_buf[slot, pl.ds((e % 4) * TQ + u * CH, CH), :], x_buf[pl.ds(r0, CH), :])
                track(r0, r, None)
                if u == NCH - 1:
                    cp_out(e).start()
            pending = [(e, u, 2) for e in range(NQ - 8, NQ - 4) for u in range(NCH)]
            for w in range(DS):
                og = load_o((NITEMS - 1) % 2, w * RS, RS)
                for n in range(NDT):
                    att_buf[3, pl.ds(w * RS, RS), n * 128:(n + 1) * 128] += _dot(og, wld(wo_buf, 3, n))
                    for _ in range(DPER):
                        if pending:
                            chunk(*pending.pop(0))
                for r0 in range(w * RS, (w + 1) * RS, CH):
                    pending.append((NQ - 4 + r0 // TQ, (r0 % TQ) // CH, 3))
            for c_ in pending:
                chunk(*c_)

        with scope('tail_a'):
            bv = best_v[...]
            mxv = jnp.max(bv, axis=0, keepdims=True)
            idxv = jnp.min(jnp.where(bv == mxv, best_i[...], S - 1), axis=0, keepdims=True)
            idx = jnp.clip(idxv[0, 0], 0, S - 1)
            base = pl.multiple_of(_shr(idx, 4) * 16, 16)
            x1f = x_buf[pl.ds(base, 16), :].astype(f32)
            if H2BUF:
                h2b = h2_buf[pl.ds(base, 16), :]
            else:
                h2b = (_ln(x1f) * (1.0 + modrow(4)) + modrow(3)).astype(bf16)
            h2 = h2b.astype(f32)
            G_ffn.wait()
        with scope('tail_gu'):
            acts = []
            for n in range(NFT):
                g_ = _dot(h2b, wg_buf[:, n * 128:(n + 1) * 128])
                u_ = _dot(h2b, wu_buf[:, n * 128:(n + 1) * 128])
                acts.append((g_ * jax.nn.sigmoid(g_) * u_).astype(bf16))
            a_ = jnp.concatenate(acts, axis=1)
        with scope('tail_d'):
            y = jnp.concatenate([_dot(a_, wd_buf[:, n * 128:(n + 1) * 128]) for n in range(NDT)], axis=1)
            y = y * jax.nn.sigmoid(mxv)
            rid = base + jax.lax.broadcasted_iota(i32, (16, 1), 0)
            upd = jnp.where(rid == idx, y, h2 * 0.0)
        with scope('tail_fin'):
            copy(out_buf.at[pl.ds(0, S)], out_hbm, s_out).wait()
            out_buf[pl.ds(base, 16), :] = (x1f + modrow(5) * (h2 + upd)).astype(bf16)
            fin = copy(out_buf.at[pl.ds(base, 16)], out_hbm.at[pl.ds(base, 16)], s_fin)
            fin.start()
            fin.wait()

    NSEM = 48

    def fn(A_x, A_k_cache, A_v_cache, A_wq, A_wo, B_x, B_w_r, B_w_gate, B_w_up, B_w_down, c, w_mod):
        x2 = A_x.reshape(S, D)
        k3 = A_k_cache.reshape(HKV, SK, DH)
        v3 = A_v_cache.reshape(HKV, SK, DH)
        hbm = pl.BlockSpec(memory_space=pl.ANY)
        out = pl.pallas_call(
            kernel,
            out_shape=jax.ShapeDtypeStruct((S, D), bf16),
            in_specs=[hbm] * 11,
            out_specs=hbm,
            scratch_shapes=[
                pltpu.VMEM((S + TQ, D), bf16),
                pltpu.VMEM((HKV, W, DH), bf16),
                pltpu.VMEM((HKV, W, DH), bf16),
                pltpu.VMEM((HQ, D, 128), bf16),
                pltpu.VMEM((HKV, NDT, 1024, 128), bf16),
                pltpu.VMEM((D, F), bf16),
                pltpu.VMEM((D, F), bf16),
                pltpu.VMEM((F, D + PADW), bf16),
                pltpu.VMEM((D, 6 * D + PADW), bf16),
                pltpu.VMEM((6, 8, D), f32),
                pltpu.VMEM((4, NDT, TM, 128), bf16),
                pltpu.VMEM((2, REP, TM, 128), bf16),
                pltpu.VMEM((4, TM, D), f32),
                pltpu.VMEM((S + TQ, D), bf16),
                pltpu.VMEM((S + TQ, D), bf16),
                pltpu.VMEM((CH, 1), f32),
                pltpu.VMEM((CH, 1), i32),
                pltpu.VMEM((1, D), bf16),
                pltpu.VMEM((D,), bf16),
                pltpu.SemaphoreType.DMA((NSEM,)),
            ],
            compiler_params=pltpu.CompilerParams(vmem_limit_bytes=126 * 1024 * 1024, flags=flags),
        )(x2, k3, v3, A_wq, A_wo, B_w_r, B_w_gate, B_w_up, B_w_down, c, w_mod)
        return out.reshape(1, S, D)

    return jax.jit(fn)


_impl = make(ORDER='G', WQW=((0, 1), (1, 2), (2, 4), (4, 8)))


@jax.jit
def pallas_adaLN_cond__sliding_block_cached__moe_arch_mod__prompt_kernel(
    A_x, A_k_cache, A_v_cache, A_wq, A_wo, B_x, B_w_r, B_w_gate, B_w_up, B_w_down, c, w_mod,
):
    return _impl(A_x, A_k_cache, A_v_cache, A_wq, A_wo, B_x, B_w_r, B_w_gate, B_w_up, B_w_down, c, w_mod)
```

```python
import jax
import jax.numpy as jnp
import jax.experimental.pallas as pl
import jax.experimental.pallas.tpu as pltpu

S, D, HQ, HKV, DH, SK, W, F = 2048, 1024, 32, 4, 128, 2048, 512, 3584
REP = HQ // HKV
LOG2E = 1.4426950408889634
SCALE = DH ** -0.5
EPS = 1e-5
bf16 = jnp.bfloat16
f32 = jnp.float32
i32 = jnp.int32
NT = (((1,), (1,)), ((), ()))

TM = 256
NB = S // TM
NDT = D // 128
NFT = F // 128
TQ = TM // 4
NQ = S // TQ
NITEMS = NB * HKV
CH = 16
NCH = TQ // CH
MODC = 4
PADW = 128
WQ0 = ((0, 1), (1, 2), (2, 4), (4, 8))
NSEM = 48


def _ln(xf):
    m = jnp.mean(xf, axis=-1, keepdims=True)
    xc = xf - m
    v = jnp.mean(xc * xc, axis=-1, keepdims=True)
    return xc * jax.lax.rsqrt(v + EPS)


def _dot(a, b):
    return jnp.dot(a, b, preferred_element_type=f32)


def _shr(x, n):
    return x >> n if isinstance(x, int) else jax.lax.shift_right_logical(x, n)


def _mult(x, n):
    return x if isinstance(x, int) else pl.multiple_of(x, n)


def _kernel(x_hbm, k_hbm, v_hbm, wq_hbm, wo_hbm, wr_hbm, wg_hbm, wu_hbm, wd_hbm, c_hbm, wmod_hbm,
            out_hbm,
            x_buf, k_buf, v_buf, wq_buf, wo_buf, wg_buf, wu_buf, wd_buf, wmod_buf, mod_buf,
            h_buf, o_buf, att_buf, out_buf, h2_buf, best_v, best_i, c_ref, wr_ref, wrf_buf, sems):
    nsem = [0]

    def new_sem():
        nsem[0] += 1
        return nsem[0] - 1

    def copy(src, dst, sem):
        return pltpu.make_async_copy(src, dst, sems.at[sem])

    class Group:
        def __init__(self, fn):
            self.cps = fn(new_sem())

        def start(self):
            for c_ in self.cps:
                c_.start()

        def wait(self):
            for c_ in self.cps:
                c_.wait()

    def wld(ref, *idx):
        return pltpu.bitcast(ref.bitcast(jnp.uint32)[idx], bf16)

    def g_x(r0, r1):
        return Group(lambda s: [copy(x_hbm.at[pl.ds(r0, r1 - r0)], x_buf.at[pl.ds(r0, r1 - r0)], s)])

    def g_wq(t0, t1):
        return Group(lambda s: [copy(wq_hbm.at[:, pl.ds(t * 128, 128)], wq_buf.at[t], s) for t in range(t0, t1)])

    def g_wo(g):
        return Group(lambda s: [copy(wo_hbm.at[pl.ds(g * 1024, 1024), pl.ds(n * 128, 128)], wo_buf.at[g, n], s)
                                for n in range(NDT)])

    def g_k(g):
        return Group(lambda s: [copy(k_hbm.at[g, pl.ds(SK - W, W), :], k_buf.at[g], s)])

    def g_v(g):
        return Group(lambda s: [copy(v_hbm.at[g, pl.ds(SK - W, W), :], v_buf.at[g], s)])

    def g_wmod(c0, c1):
        return Group(lambda s: [copy(wmod_hbm.at[:, pl.ds(c0, c1 - c0)], wmod_buf.at[:, pl.ds(c0, c1 - c0)], s)])

    G_c = Group(lambda s: [copy(c_hbm, c_ref, s)])
    G_wr = Group(lambda s: [copy(wr_hbm, wr_ref, s)])
    G_x0, G_x1 = g_x(0, TM), g_x(TM, 2 * TM)
    G_xa, G_xb, G_xc = g_x(2 * TM, 2 * TM + TQ), g_x(2 * TM + TQ, 4 * TM), g_x(4 * TM, S)
    G_mod0 = [g_wmod(i * 2048 // MODC, (i + 1) * 2048 // MODC) for i in range(MODC)]
    G_mod12 = g_wmod(2048, 6144)
    G_wq0 = [g_wq(a, b) for a, b in WQ0]
    G_wq = [None] + [g_wq(8 * g, 8 * g + 8) for g in range(1, HKV)]
    G_k = [g_k(g) for g in range(HKV)]
    G_v = [g_v(g) for g in range(HKV)]
    G_wo = [g_wo(g) for g in range(HKV)]
    G_ffn = Group(lambda s: [copy(wg_hbm, wg_buf, s), copy(wu_hbm, wu_buf, s),
                             copy(wd_hbm, wd_buf.at[:, pl.ds(0, D)], s)])
    s_out = new_sem()
    s_fin = new_sem()
    assert nsem[0] <= NSEM

    def cp_out(e):
        r0 = _mult(e * TQ, TQ)
        return copy(out_buf.at[pl.ds(r0, TQ)], out_hbm.at[pl.ds(r0, TQ)], s_out)

    first_order = [G_c, G_x0] + G_mod0 + [G_wq0[0], G_wq0[1], G_k[0], G_v[0]] + G_wq0[2:] + [G_x1, G_wr]
    first_order += [G_wo[0], G_xa, G_wq[1], G_k[1], G_v[1], G_xb, G_wo[1], G_wq[2], G_k[2], G_v[2], G_wo[2]]
    later_order = [G_wq[3], G_k[3], G_v[3], G_wo[3], G_mod12, G_xc, G_ffn]
    for grp in first_order:
        grp.start()

    def modrow(i, nrows):
        return jnp.concatenate([mod_buf[i]] * (nrows // 8), axis=0)

    def normalize(xv):
        return _ln(xv.astype(f32))

    def store_h(hn, slot, hr0, nrows):
        h = (hn * modrow(1, nrows) + modrow(0, nrows)).astype(bf16)
        for c in range(NDT):
            h_buf[slot, c, pl.ds(hr0, nrows), :] = h[:, c * 128:(c + 1) * 128]

    def load_h(slot):
        return jnp.concatenate([h_buf[slot, c] for c in range(NDT)], axis=1)

    def qproj(t, hv):
        return (_dot(hv, wld(wq_buf, t)) * (SCALE * LOG2E)).astype(bf16)

    def qk(g, qh):
        return jax.lax.dot_general(qh, wld(k_buf, g), NT, preferred_element_type=f32)

    def softmax(s):
        m = jnp.max(s, axis=-1, keepdims=True)
        p = jnp.exp2(s - m)
        l = jnp.sum(p, axis=-1, keepdims=True)
        r = pl.reciprocal(l, approx=True)
        r = r * (2.0 - l * r)
        return p.astype(bf16), r

    def pv(g, p, r):
        return (_dot(p, wld(v_buf, g)) * r).astype(bf16)

    def load_o(slot, r0=0, nrows=TM):
        return jnp.concatenate([o_buf[slot, j, pl.ds(r0, nrows), :] for j in range(REP)], axis=1)

    def epilogue(r0, att, xv):
        x1 = (xv.astype(f32) + modrow(2, CH) * att).astype(bf16)
        x_buf[pl.ds(r0, CH), :] = x1
        x1f = x1.astype(f32)
        h2b = (_ln(x1f) * modrow(4, CH) + modrow(3, CH)).astype(bf16)
        h2_buf[pl.ds(r0, CH), :] = h2b
        h2 = h2b.astype(f32)
        wr = jnp.concatenate([wrf_buf[...]] * (CH // 8), axis=0)
        r = jnp.sum(h2 * wr, axis=-1, keepdims=True)
        out_buf[pl.ds(r0, CH), :] = (x1f + modrow(5, CH) * (h2 + h2 * 0.0)).astype(bf16)
        return r

    def track(r0, r, valid):
        rid = r0 + jax.lax.broadcasted_iota(i32, (CH, 1), 0)
        bv = best_v[...]
        upd = r > bv
        if valid is not None:
            upd = jnp.logical_and(upd, valid)
        best_i[...] = jnp.where(upd, rid, best_i[...])
        best_v[...] = jnp.where(upd, r, bv)

    def mod_tiles(sc8, n0, n1):
        for n in range(n0, n1):
            d = _dot(sc8, wmod_buf[:, n * 128:(n + 1) * 128]).astype(bf16).astype(f32)
            if n // 8 in (1, 4):
                d = 1.0 + d
            mod_buf[n // 8, :, (n % 8) * 128:(n % 8 + 1) * 128] = d

    att_buf[...] = jnp.zeros(att_buf.shape, f32)
    x_buf[pl.ds(S, TQ), :] = jnp.zeros((TQ, D), bf16)
    mod_buf[...] = jnp.zeros(mod_buf.shape, f32)
    best_v[...] = jnp.full(best_v.shape, -jnp.inf, f32)
    best_i[...] = jnp.zeros(best_i.shape, i32)

    G_c.wait()
    cf = c_ref[...].astype(f32)
    sc8 = jnp.broadcast_to((cf * jax.nn.sigmoid(cf)).astype(bf16), (8, D))
    G_x0.wait()
    hn0 = normalize(x_buf[pl.ds(0, TM), :])
    for i in range(MODC):
        G_mod0[i].wait()
        mod_tiles(sc8, i * 16 // MODC, (i + 1) * 16 // MODC)
    store_h(hn0, 0, 0, TM)

    def item(i, first, steady=False):
        par = i & 1
        g = _shr(i, 1) & 3
        pair = _shr(i, 3)
        hslot = (pair & 1) * 2 + par
        ip = i - 1
        gp = _shr(ip, 1) & 3
        aslot = (_shr(ip, 3) & 1) * 2 + (ip & 1)
        if not first:
            u_ln = ip & 7
            pn = _shr(ip, 3) + 1
            lr0 = _mult(jnp.minimum(pn * 8 + u_ln, NQ - 1) * TQ, TQ)
            lslot = (pn & 1) * 2 + _shr(u_ln, 2)
            lh0 = (u_ln & 3) * TQ
            e = i - 8
            valid = e >= 0
            ec = jnp.maximum(e, 0)
            er0 = _mult(jnp.where(valid, e, NQ) * TQ, TQ)
            eslot = _shr(ec, 2) & 3
            ea0 = _mult((ec & 3) * TQ, TQ)

        if steady:
            cp_out(e - 1).start()
        elif not first:
            for k_, grps in ((1, [G_wo[0], G_xa, G_wr]), (2, [G_wq[1], G_k[1], G_v[1], G_xb]), (3, [G_wo[1]]),
                             (4, [G_wq[2], G_k[2], G_v[2]]), (5, [G_wo[2]]), (6, [G_wq[3], G_k[3], G_v[3]]),
                             (7, [G_wo[3], G_mod12]), (8, [G_xc])):
                @pl.when(i == k_)
                def _():
                    for grp in grps:
                        grp.wait()
                    if k_ == 1:
                        wrf_buf[...] = jnp.broadcast_to(wr_ref[...].astype(f32).reshape(1, D), (8, D))
                    if k_ == 7:
                        mod_tiles(sc8, 16, 48)

        hv = load_h(hslot)
        if not first:
            og = load_o(1 - par)
            xl = x_buf[pl.ds(lr0, TQ), :]
            xe = x_buf[pl.ds(er0, TQ), :]
            ae = att_buf[eslot, pl.ds(ea0, TQ), :]

        def do_ln(u):
            store_h(normalize(xl[u * CH:(u + 1) * CH]), lslot, _mult(lh0 + u * CH, CH), CH)

        def do_epi(u):
            r0 = _mult(er0 + u * CH, CH)
            track(r0, epilogue(r0, ae[u * CH:(u + 1) * CH], xe[u * CH:(u + 1) * CH]), valid)

        def qp(j):
            if first:
                for grp, (a, _) in zip(G_wq0, WQ0):
                    if a == j:
                        grp.wait()
            return qproj(g * REP + j, hv)

        qs = {0: qp(0), 1: qp(1)}
        if first:
            G_k[0].wait()
        ss = {0: qk(g, qs.pop(0))}
        for j in range(REP):
            if j + 1 < REP:
                ss[j + 1] = qk(g, qs.pop(j + 1))
            if not first:
                if j < NCH:
                    do_ln(j)
                else:
                    do_epi(j - NCH)
            else:
                if j == 1:
                    for grp in later_order:
                        grp.start()
                if j == 4:
                    G_x1.wait()
                if j >= 4:
                    r0 = (j - 4) * TQ
                    store_h(normalize(x_buf[pl.ds(TM + r0, TQ), :]), 1, r0, TQ)
            if j + 2 < REP:
                qs[j + 2] = qp(j + 2)
            if not first:
                c = _dot(og, wld(wo_buf, gp, j))
                old = att_buf[aslot, :, j * 128:(j + 1) * 128]
                att_buf[aslot, :, j * 128:(j + 1) * 128] = jnp.where(gp == 0, 0.0, old) + c
            p, r = softmax(ss.pop(j))
            if first and j == 0:
                G_v[0].wait()
            o_buf[par, j] = pv(g, p, r)

    item(0, True)

    def early_body(i, carry):
        item(i, False)
        return carry

    def steady_body(i, carry):
        item(i, False, True)
        return carry

    jax.lax.fori_loop(1, 9, early_body, 0)
    jax.lax.fori_loop(9, NITEMS, steady_body, 0)

    cp_out(NQ - 9).start()

    def chunk(e, u, slot):
        r0 = e * TQ + u * CH
        r = epilogue(r0, att_buf[slot, pl.ds((e % 4) * TQ + u * CH, CH), :], x_buf[pl.ds(r0, CH), :])
        track(r0, r, None)
        if u == NCH - 1:
            cp_out(e).start()

    pending = [(e, u, 2) for e in range(NQ - 8, NQ - 4) for u in range(NCH)]
    for w in range(4):
        og = load_o((NITEMS - 1) % 2, w * TQ, TQ)
        for n in range(NDT):
            att_buf[3, pl.ds(w * TQ, TQ), n * 128:(n + 1) * 128] += _dot(og, wld(wo_buf, 3, n))
            if pending:
                chunk(*pending.pop(0))
        pending += [(NQ - 4 + w, u, 3) for u in range(NCH)]
    for c_ in pending:
        chunk(*c_)

    bv = best_v[...]
    mxv = jnp.max(bv, axis=0, keepdims=True)
    idxv = jnp.min(jnp.where(bv == mxv, best_i[...], S - 1), axis=0, keepdims=True)
    idx = jnp.clip(idxv[0, 0], 0, S - 1)
    base = pl.multiple_of(_shr(idx, 4) * 16, 16)
    x1f = x_buf[pl.ds(base, 16), :].astype(f32)
    h2b = h2_buf[pl.ds(base, 16), :]
    h2 = h2b.astype(f32)
    G_ffn.wait()
    acts = []
    for n in range(NFT):
        g_ = _dot(h2b, wg_buf[:, n * 128:(n + 1) * 128])
        u_ = _dot(h2b, wu_buf[:, n * 128:(n + 1) * 128])
        acts.append((g_ * jax.nn.sigmoid(g_) * u_).astype(bf16))
    a_ = jnp.concatenate(acts, axis=1)
    y = jnp.concatenate([_dot(a_, wd_buf[:, n * 128:(n + 1) * 128]) for n in range(NDT)], axis=1)
    y = y * jax.nn.sigmoid(mxv)
    rid = base + jax.lax.broadcasted_iota(i32, (16, 1), 0)
    upd = jnp.where(rid == idx, y, h2 * 0.0)
    copy(out_buf.at[pl.ds(0, S)], out_hbm, s_out).wait()
    out_buf[pl.ds(base, 16), :] = (x1f + modrow(5, 16) * (h2 + upd)).astype(bf16)
    fin = copy(out_buf.at[pl.ds(base, 16)], out_hbm.at[pl.ds(base, 16)], s_fin)
    fin.start()
    fin.wait()


_SCRATCH = [
    pltpu.VMEM((S + TQ, D), bf16),
    pltpu.VMEM((HKV, W, DH), bf16),
    pltpu.VMEM((HKV, W, DH), bf16),
    pltpu.VMEM((HQ, D, 128), bf16),
    pltpu.VMEM((HKV, NDT, 1024, 128), bf16),
    pltpu.VMEM((D, F), bf16),
    pltpu.VMEM((D, F), bf16),
    pltpu.VMEM((F, D + PADW), bf16),
    pltpu.VMEM((D, 6 * D + PADW), bf16),
    pltpu.VMEM((6, 8, D), f32),
    pltpu.VMEM((4, NDT, TM, 128), bf16),
    pltpu.VMEM((2, REP, TM, 128), bf16),
    pltpu.VMEM((4, TM, D), f32),
    pltpu.VMEM((S + TQ, D), bf16),
    pltpu.VMEM((S + TQ, D), bf16),
    pltpu.VMEM((CH, 1), f32),
    pltpu.VMEM((CH, 1), i32),
    pltpu.VMEM((1, D), bf16),
    pltpu.VMEM((D,), bf16),
    pltpu.VMEM((8, D), f32),
    pltpu.SemaphoreType.DMA((NSEM,)),
]


@jax.jit
def pallas_adaLN_cond__sliding_block_cached__moe_arch_mod__prompt_kernel(
    A_x: jax.Array,
    A_k_cache: jax.Array,
    A_v_cache: jax.Array,
    A_wq: jax.Array,
    A_wo: jax.Array,
    B_x: jax.Array,
    B_w_r: jax.Array,
    B_w_gate: jax.Array,
    B_w_up: jax.Array,
    B_w_down: jax.Array,
    c: jax.Array,
    w_mod: jax.Array,
):
    del B_x
    hbm = pl.BlockSpec(memory_space=pl.ANY)
    out = pl.pallas_call(
        _kernel,
        out_shape=jax.ShapeDtypeStruct((S, D), bf16),
        in_specs=[hbm] * 11,
        out_specs=hbm,
        scratch_shapes=_SCRATCH,
        compiler_params=pltpu.CompilerParams(vmem_limit_bytes=126 * 1024 * 1024),
    )(A_x.reshape(S, D), A_k_cache.reshape(HKV, SK, DH), A_v_cache.reshape(HKV, SK, DH), A_wq, A_wo,
      B_w_r, B_w_gate, B_w_up, B_w_down, c, w_mod)
    return out.reshape(1, S, D)
```

```python
import jax
import jax.numpy as jnp
import jax.experimental.pallas as pl
import jax.experimental.pallas.tpu as pltpu

S, D, HQ, HKV, DH, SK, W, F = 2048, 1024, 32, 4, 128, 2048, 512, 3584
REP = HQ // HKV
LOG2E = 1.4426950408889634
SCALE = DH ** -0.5
EPS = 1e-5
bf16 = jnp.bfloat16
f32 = jnp.float32
i32 = jnp.int32
NT = (((1,), (1,)), ((), ()))

TM = 256
NB = S // TM
NDT = D // 128
NFT = F // 128
TQ = TM // 4
NQ = S // TQ
NITEMS = NB * HKV
CH = 16
NCH = TQ // CH
MODC = 4
PADW = 128
WQ0 = ((0, 1), (1, 2), (2, 4), (4, 8))
NSEM = 48


def _ln(xf):
    m = jnp.mean(xf, axis=-1, keepdims=True)
    xc = xf - m
    v = jnp.mean(xc * xc, axis=-1, keepdims=True)
    return xc * jax.lax.rsqrt(v + EPS)


def _dot(a, b):
    return jnp.dot(a, b, preferred_element_type=f32)


def _shr(x, n):
    return x >> n if isinstance(x, int) else jax.lax.shift_right_logical(x, n)


def _mult(x, n):
    return x if isinstance(x, int) else pl.multiple_of(x, n)


def _kernel(x_hbm, k_hbm, v_hbm, wq_hbm, wo_hbm, wr_hbm, wg_hbm, wu_hbm, wd_hbm, c_hbm, wmod_hbm,
            out_hbm,
            x_buf, k_buf, v_buf, wq_buf, wo_buf, wg_buf, wu_buf, wd_buf, wmod_buf, mod_buf,
            h_buf, o_buf, att_buf, out_buf, h2_buf, scol_buf, best_v, best_i, c_ref, wr_ref, wrf_buf, sems):
    nsem = [0]

    def new_sem():
        nsem[0] += 1
        return nsem[0] - 1

    def copy(src, dst, sem):
        return pltpu.make_async_copy(src, dst, sems.at[sem])

    class Group:
        def __init__(self, fn):
            self.cps = fn(new_sem())

        def start(self):
            for c_ in self.cps:
                c_.start()

        def wait(self):
            for c_ in self.cps:
                c_.wait()

    def wld(ref, *idx):
        return pltpu.bitcast(ref.bitcast(jnp.uint32)[idx], bf16)

    def g_x(r0, r1):
        return Group(lambda s: [copy(x_hbm.at[pl.ds(r0, r1 - r0)], x_buf.at[pl.ds(r0, r1 - r0)], s)])

    def g_wq(t0, t1):
        return Group(lambda s: [copy(wq_hbm.at[:, pl.ds(t * 128, 128)], wq_buf.at[t], s) for t in range(t0, t1)])

    def g_wo(g):
        return Group(lambda s: [copy(wo_hbm.at[pl.ds(g * 1024, 1024), pl.ds(n * 128, 128)], wo_buf.at[g, n], s)
                                for n in range(NDT)])

    def g_k(g):
        return Group(lambda s: [copy(k_hbm.at[g, pl.ds(SK - W, W), :], k_buf.at[g], s)])

    def g_v(g):
        return Group(lambda s: [copy(v_hbm.at[g, pl.ds(SK - W, W), :], v_buf.at[g], s)])

    def g_wmod(c0, c1):
        return Group(lambda s: [copy(wmod_hbm.at[:, pl.ds(c0, c1 - c0)], wmod_buf.at[:, pl.ds(c0, c1 - c0)], s)])

    G_c = Group(lambda s: [copy(c_hbm, c_ref, s)])
    G_wr = Group(lambda s: [copy(wr_hbm, wr_ref, s)])
    G_x0, G_x1 = g_x(0, TM), g_x(TM, 2 * TM)
    G_xa, G_xb, G_xc = g_x(2 * TM, 2 * TM + TQ), g_x(2 * TM + TQ, 4 * TM), g_x(4 * TM, S)
    G_mod0 = [g_wmod(i * 2048 // MODC, (i + 1) * 2048 // MODC) for i in range(MODC)]
    G_modv = {k: g_wmod(2048 + (k - 2) * 768, min(2048 + (k - 1) * 768, 6144)) for k in range(2, 8)}
    G_wq0 = [g_wq(a, b) for a, b in WQ0]
    G_wq = [None] + [g_wq(8 * g, 8 * g + 8) for g in range(1, HKV)]
    G_k = [g_k(g) for g in range(HKV)]
    G_v = [g_v(g) for g in range(HKV)]
    G_wo = [g_wo(g) for g in range(HKV)]
    G_ffn = Group(lambda s: [copy(wg_hbm, wg_buf, s), copy(wu_hbm, wu_buf, s),
                             copy(wd_hbm, wd_buf.at[:, pl.ds(0, D)], s)])
    s_out = new_sem()
    s_fin = new_sem()
    assert nsem[0] <= NSEM

    def cp_out(e):
        r0 = _mult(e * TQ, TQ)
        return copy(out_buf.at[pl.ds(r0, TQ)], out_hbm.at[pl.ds(r0, TQ)], s_out)

    first_order = [G_c, G_x0] + G_mod0 + [G_wq0[0], G_wq0[1], G_k[0], G_v[0]] + G_wq0[2:] + [G_x1, G_wr]
    first_order += [G_wo[0], G_xa, G_wq[1], G_k[1], G_v[1], G_xb, G_modv[2], G_wo[1], G_modv[3],
                    G_wq[2], G_k[2], G_v[2], G_modv[4], G_wo[2]]
    later_order = [G_modv[5], G_wq[3], G_k[3], G_v[3], G_modv[6], G_wo[3], G_modv[7], G_xc, G_ffn]
    for grp in first_order:
        grp.start()

    def modrow(i, nrows):
        return jnp.concatenate([mod_buf[i]] * (nrows // 8), axis=0)

    def normalize(xv):
        return _ln(xv.astype(f32))

    def store_h(hn, slot, hr0, nrows):
        h = (hn * modrow(1, nrows) + modrow(0, nrows)).astype(bf16)
        for c in range(NDT):
            h_buf[slot, c, pl.ds(hr0, nrows), :] = h[:, c * 128:(c + 1) * 128]

    def load_h(slot):
        return jnp.concatenate([h_buf[slot, c] for c in range(NDT)], axis=1)

    def qproj(t, hv):
        return (_dot(hv, wld(wq_buf, t)) * (SCALE * LOG2E)).astype(bf16)

    def qk(g, qh):
        return jax.lax.dot_general(qh, wld(k_buf, g), NT, preferred_element_type=f32)

    def softmax(s):
        m = jnp.max(s, axis=-1, keepdims=True)
        p = jnp.exp2(s - m)
        l = jnp.sum(p, axis=-1, keepdims=True)
        r = pl.reciprocal(l, approx=True)
        r = r * (2.0 - l * r)
        return p.astype(bf16), r

    def pv(g, p, r):
        return (_dot(p, wld(v_buf, g)) * r).astype(bf16)

    def load_o(slot, r0=0, nrows=TM):
        return jnp.concatenate([o_buf[slot, j, pl.ds(r0, nrows), :] for j in range(REP)], axis=1)

    def epilogue(r0, att, xv):
        x1 = (xv.astype(f32) + modrow(2, CH) * att).astype(bf16)
        x_buf[pl.ds(r0, CH), :] = x1
        x1f = x1.astype(f32)
        h2b = (_ln(x1f) * modrow(4, CH) + modrow(3, CH)).astype(bf16)
        h2_buf[pl.ds(r0, CH), :] = h2b
        h2 = h2b.astype(f32)
        wr = jnp.concatenate([wrf_buf[...]] * (CH // 8), axis=0)
        r = jnp.sum(h2 * wr, axis=-1, keepdims=True)
        out_buf[pl.ds(r0, CH), :] = (x1f + modrow(5, CH) * (h2 + h2 * 0.0)).astype(bf16)
        return r

    def track(r0, r):
        rid = r0 + jax.lax.broadcasted_iota(i32, (CH, 1), 0)
        bv = best_v[...]
        upd = r > bv
        best_i[...] = jnp.where(upd, rid, best_i[...])
        best_v[...] = jnp.where(upd, r, bv)

    def mod_tiles(sc8, n0, n1):
        for n in range(n0, n1):
            d = _dot(sc8, wmod_buf[:, n * 128:(n + 1) * 128]).astype(bf16).astype(f32)
            if n // 8 in (1, 4):
                d = 1.0 + d
            mod_buf[n // 8, :, (n % 8) * 128:(n % 8 + 1) * 128] = d

    att_buf[...] = jnp.zeros(att_buf.shape, f32)
    mod_buf[...] = jnp.zeros(mod_buf.shape, f32)
    best_v[...] = jnp.full(best_v.shape, -jnp.inf, f32)
    best_i[...] = jnp.zeros(best_i.shape, i32)

    G_c.wait()
    cf = c_ref[...].astype(f32)
    sc8 = jnp.broadcast_to((cf * jax.nn.sigmoid(cf)).astype(bf16), (8, D))
    scf = sc8[0:1].astype(f32)
    for c_ in range(NDT):
        scol_buf[c_ * 128:(c_ + 1) * 128, :] = jnp.broadcast_to(scf[:, c_ * 128:(c_ + 1) * 128], (128, 128)).T
    G_x0.wait()
    hn0 = normalize(x_buf[pl.ds(0, TM), :])
    for i in range(MODC):
        G_mod0[i].wait()
        mod_tiles(sc8, i * 16 // MODC, (i + 1) * 16 // MODC)
    store_h(hn0, 0, 0, TM)

    def item(i, first, steady=False):
        par = i & 1
        g = _shr(i, 1) & 3
        pair = _shr(i, 3)
        hslot = (pair & 1) * 2 + par
        ip = i - 1
        gp = _shr(ip, 1) & 3
        aslot = (_shr(ip, 3) & 1) * 2 + (ip & 1)
        if not first:
            u_ln = ip & 7
            pn = _shr(ip, 3) + 1
            lr0 = _mult(jnp.minimum(pn * 8 + u_ln, NQ - 1) * TQ, TQ)
            lslot = (pn & 1) * 2 + _shr(u_ln, 2)
            lh0 = (u_ln & 3) * TQ
            e = i - 8
            er0 = _mult(e * TQ, TQ)
            eslot = _shr(e, 2) & 3
            ea0 = _mult((e & 3) * TQ, TQ)

        if not first and not steady:
            for k_, grps in ((1, [G_wo[0], G_xa, G_wr]), (2, [G_wq[1], G_k[1], G_v[1], G_xb]), (3, [G_wo[1]]),
                             (4, [G_wq[2], G_k[2], G_v[2]]), (5, [G_wo[2]]), (6, [G_wq[3], G_k[3], G_v[3]]),
                             (7, [G_wo[3]])):
                @pl.when(i == k_)
                def _():
                    for grp in grps:
                        grp.wait()
                    if k_ == 1:
                        wrf_buf[...] = jnp.broadcast_to(wr_ref[...].astype(f32).reshape(1, D), (8, D))
                    if k_ >= 2:
                        G_modv[k_].wait()

        hv = load_h(hslot)
        if not first:
            og = load_o(1 - par)
            xl = x_buf[pl.ds(lr0, TQ), :]
            if steady:
                xe = x_buf[pl.ds(er0, TQ), :]
                ae = att_buf[eslot, pl.ds(ea0, TQ), :]

        def do_ln(u):
            store_h(normalize(xl[u * CH:(u + 1) * CH]), lslot, _mult(lh0 + u * CH, CH), CH)

        def do_epi(u):
            r0 = _mult(er0 + u * CH, CH)
            track(r0, epilogue(r0, ae[u * CH:(u + 1) * CH], xe[u * CH:(u + 1) * CH]))

        early = not first and not steady
        if early:
            mv_n = [16 + (i - 2) * 6 + u for u in range(6)]
            mv_valid = [jnp.logical_and(i >= 2, n_ < 48) for n_ in mv_n]
            mv_src = [pl.multiple_of(jnp.where(v_, n_, 0) * 128, 128) for v_, n_ in zip(mv_valid, mv_n)]
            mv_acc = [None] * 6

        def do_modv(kk):
            col = scol_buf[kk * 128:(kk + 1) * 128, :]
            for r_ in range(0, 128, 8):
                cr = col[r_:r_ + 8]
                for u in range(6):
                    p_ = wmod_buf[kk * 128 + r_:kk * 128 + r_ + 8, pl.ds(mv_src[u], 128)].astype(f32) * cr
                    mv_acc[u] = p_ if mv_acc[u] is None else mv_acc[u] + p_

        def fin_modv():
            for u in range(6):
                d = jnp.sum(mv_acc[u], axis=0, keepdims=True).astype(bf16).astype(f32)
                n_ = mv_n[u]
                is_scale = jnp.logical_and(n_ >= 32, n_ < 40)
                d = d + jnp.where(is_scale, 1.0, 0.0)
                row = jnp.where(mv_valid[u], _shr(n_, 3), 6)
                mod_buf[row, :, pl.ds(pl.multiple_of((n_ & 7) * 128, 128), 128)] = jnp.broadcast_to(d, (8, 128))

        def qp(j):
            if first:
                for grp, (a, _) in zip(G_wq0, WQ0):
                    if a == j:
                        grp.wait()
            return qproj(g * REP + j, hv)

        qs = {0: qp(0), 1: qp(1)}
        if first:
            G_k[0].wait()
        ss = {0: qk(g, qs.pop(0))}
        for j in range(REP):
            if j + 1 < REP:
                ss[j + 1] = qk(g, qs.pop(j + 1))
            if not first:
                if j < NCH:
                    do_ln(j)
                elif steady:
                    do_epi(j - NCH)
                if early:
                    do_modv(j)
                    if j == REP - 1:
                        fin_modv()
            else:
                if j == 1:
                    for grp in later_order:
                        grp.start()
                if j == 4:
                    G_x1.wait()
                if j >= 4:
                    r0 = (j - 4) * TQ
                    store_h(normalize(x_buf[pl.ds(TM + r0, TQ), :]), 1, r0, TQ)
            if j + 2 < REP:
                qs[j + 2] = qp(j + 2)
            if not first:
                c = _dot(og, wld(wo_buf, gp, j))
                old = att_buf[aslot, :, j * 128:(j + 1) * 128]
                att_buf[aslot, :, j * 128:(j + 1) * 128] = jnp.where(gp == 0, 0.0, old) + c
            p, r = softmax(ss.pop(j))
            if first and j == 0:
                G_v[0].wait()
            o_buf[par, j] = pv(g, p, r)
        if steady:
            cp_out(e).start()

    item(0, True)

    def early_body(i, carry):
        item(i, False)
        return carry

    def steady_body(i, carry):
        item(i, False, True)
        return carry

    jax.lax.fori_loop(1, 8, early_body, 0)
    G_xc.wait()
    jax.lax.fori_loop(8, NITEMS, steady_body, 0)

    def chunk(e, u, slot):
        r0 = e * TQ + u * CH
        r = epilogue(r0, att_buf[slot, pl.ds((e % 4) * TQ + u * CH, CH), :], x_buf[pl.ds(r0, CH), :])
        track(r0, r)
        if u == NCH - 1:
            cp_out(e).start()

    pending = [(e, u, 2) for e in range(NQ - 8, NQ - 4) for u in range(NCH)]
    for w in range(4):
        og = load_o((NITEMS - 1) % 2, w * TQ, TQ)
        for n in range(NDT):
            att_buf[3, pl.ds(w * TQ, TQ), n * 128:(n + 1) * 128] += _dot(og, wld(wo_buf, 3, n))
            if pending:
                chunk(*pending.pop(0))
        pending += [(NQ - 4 + w, u, 3) for u in range(NCH)]
    for c_ in pending:
        chunk(*c_)

    bv = best_v[...]
    mxv = jnp.max(bv, axis=0, keepdims=True)
    idxv = jnp.min(jnp.where(bv == mxv, best_i[...], S - 1), axis=0, keepdims=True)
    idx = jnp.clip(idxv[0, 0], 0, S - 1)
    base = pl.multiple_of(_shr(idx, 4) * 16, 16)
    x1f = x_buf[pl.ds(base, 16), :].astype(f32)
    h2b = h2_buf[pl.ds(base, 16), :]
    h2 = h2b.astype(f32)
    G_ffn.wait()
    acts = []
    for n in range(NFT):
        g_ = _dot(h2b, wg_buf[:, n * 128:(n + 1) * 128])
        u_ = _dot(h2b, wu_buf[:, n * 128:(n + 1) * 128])
        acts.append((g_ * jax.nn.sigmoid(g_) * u_).astype(bf16))
    a_ = jnp.concatenate(acts, axis=1)
    y = jnp.concatenate([_dot(a_, wd_buf[:, n * 128:(n + 1) * 128]) for n in range(NDT)], axis=1)
    y = y * jax.nn.sigmoid(mxv)
    rid = base + jax.lax.broadcasted_iota(i32, (16, 1), 0)
    upd = jnp.where(rid == idx, y, h2 * 0.0)
    copy(out_buf, out_hbm, s_out).wait()
    out_buf[pl.ds(base, 16), :] = (x1f + modrow(5, 16) * (h2 + upd)).astype(bf16)
    fin = copy(out_buf.at[pl.ds(base, 16)], out_hbm.at[pl.ds(base, 16)], s_fin)
    fin.start()
    fin.wait()


_SCRATCH = [
    pltpu.VMEM((S, D), bf16),
    pltpu.VMEM((HKV, W, DH), bf16),
    pltpu.VMEM((HKV, W, DH), bf16),
    pltpu.VMEM((HQ, D, 128), bf16),
    pltpu.VMEM((HKV, NDT, 1024, 128), bf16),
    pltpu.VMEM((D, F), bf16),
    pltpu.VMEM((D, F), bf16),
    pltpu.VMEM((F, D + PADW), bf16),
    pltpu.VMEM((D, 6 * D + PADW), bf16),
    pltpu.VMEM((7, 8, D), f32),
    pltpu.VMEM((4, NDT, TM, 128), bf16),
    pltpu.VMEM((2, REP, TM, 128), bf16),
    pltpu.VMEM((4, TM, D), f32),
    pltpu.VMEM((S, D), bf16),
    pltpu.VMEM((S, D), bf16),
    pltpu.VMEM((D, 128), f32),
    pltpu.VMEM((CH, 1), f32),
    pltpu.VMEM((CH, 1), i32),
    pltpu.VMEM((1, D), bf16),
    pltpu.VMEM((D,), bf16),
    pltpu.VMEM((8, D), f32),
    pltpu.SemaphoreType.DMA((NSEM,)),
]


@jax.jit
def pallas_adaLN_cond__sliding_block_cached__moe_arch_mod__prompt_kernel(
    A_x: jax.Array,
    A_k_cache: jax.Array,
    A_v_cache: jax.Array,
    A_wq: jax.Array,
    A_wo: jax.Array,
    B_x: jax.Array,
    B_w_r: jax.Array,
    B_w_gate: jax.Array,
    B_w_up: jax.Array,
    B_w_down: jax.Array,
    c: jax.Array,
    w_mod: jax.Array,
):
    del B_x
    hbm = pl.BlockSpec(memory_space=pl.ANY)
    out = pl.pallas_call(
        _kernel,
        out_shape=jax.ShapeDtypeStruct((S, D), bf16),
        in_specs=[hbm] * 11,
        out_specs=hbm,
        scratch_shapes=_SCRATCH,
        compiler_params=pltpu.CompilerParams(vmem_limit_bytes=126 * 1024 * 1024),
    )(A_x.reshape(S, D), A_k_cache.reshape(HKV, SK, DH), A_v_cache.reshape(HKV, SK, DH), A_wq, A_wo,
      B_w_r, B_w_gate, B_w_up, B_w_down, c, w_mod)
    return out.reshape(1, S, D)
```

```python
import jax
import jax.numpy as jnp
import jax.experimental.pallas as pl
import jax.experimental.pallas.tpu as pltpu

S, D, HQ, HKV, DH, SK, W, F = 2048, 1024, 32, 4, 128, 2048, 512, 3584
REP = HQ // HKV
LOG2E = 1.4426950408889634
SCALE = DH ** -0.5
EPS = 1e-5
bf16 = jnp.bfloat16
f32 = jnp.float32
i32 = jnp.int32
NT = (((1,), (1,)), ((), ()))

TM = 256
NB = S // TM
NDT = D // 128
NFT = F // 128
TQ = TM // 4
NQ = S // TQ
NITEMS = NB * HKV
CH = 16
NCH = TQ // CH
MODC = 4
PADW = 128
WQ0 = ((0, 1), (1, 2), (2, 4), (4, 8))
NSEM = 48


def _ln(xf):
    m = jnp.mean(xf, axis=-1, keepdims=True)
    xc = xf - m
    v = jnp.mean(xc * xc, axis=-1, keepdims=True)
    return xc * jax.lax.rsqrt(v + EPS)


def _dot(a, b):
    return jnp.dot(a, b, preferred_element_type=f32)


def _shr(x, n):
    return x >> n if isinstance(x, int) else jax.lax.shift_right_logical(x, n)


def _mult(x, n):
    return x if isinstance(x, int) else pl.multiple_of(x, n)


def _kernel(x_hbm, k_hbm, v_hbm, wq_hbm, wo_hbm, wr_hbm, wg_hbm, wu_hbm, wd_hbm, c_hbm, wmod_hbm,
            out_hbm,
            x_buf, k_buf, v_buf, wq_buf, wo_buf, wg_buf, wu_buf, wd_buf, wmod_buf, mod_buf,
            h_buf, o_buf, att_buf, out_buf, h2_buf, scol_buf, best_v, best_i, c_ref, wr_ref, wrf_buf, sems):
    nsem = [0]

    def new_sem():
        nsem[0] += 1
        return nsem[0] - 1

    def copy(src, dst, sem):
        return pltpu.make_async_copy(src, dst, sems.at[sem])

    class Group:
        def __init__(self, fn):
            self.cps = fn(new_sem())

        def start(self):
            for c_ in self.cps:
                c_.start()

        def wait(self):
            for c_ in self.cps:
                c_.wait()

    def g_x(r0, r1):
        return Group(lambda s: [copy(x_hbm.at[pl.ds(r0, r1 - r0)], x_buf.at[pl.ds(r0, r1 - r0)], s)])

    def g_wq(t0, t1):
        return Group(lambda s: [copy(wq_hbm.at[:, pl.ds(t * 128, 128)], wq_buf.at[t], s) for t in range(t0, t1)])

    def g_wo(g):
        return Group(lambda s: [copy(wo_hbm.at[pl.ds(g * 1024, 1024), pl.ds(n * 128, 128)], wo_buf.at[g, n], s)
                                for n in range(NDT)])

    def g_k(g):
        return Group(lambda s: [copy(k_hbm.at[g, pl.ds(SK - W, W), :], k_buf.at[g], s)])

    def g_v(g):
        return Group(lambda s: [copy(v_hbm.at[g, pl.ds(SK - W, W), :], v_buf.at[g], s)])

    def g_wmod(c0, c1):
        return Group(lambda s: [copy(wmod_hbm.at[:, pl.ds(c0, c1 - c0)], wmod_buf.at[:, pl.ds(c0, c1 - c0)], s)])

    G_c = Group(lambda s: [copy(c_hbm, c_ref, s)])
    G_wr = Group(lambda s: [copy(wr_hbm, wr_ref, s)])
    G_x0, G_x1 = g_x(0, TM), g_x(TM, 2 * TM)
    G_xa, G_xb, G_xc = g_x(2 * TM, 2 * TM + TQ), g_x(2 * TM + TQ, 4 * TM), g_x(4 * TM, S)
    G_mod0 = [g_wmod(i * 2048 // MODC, (i + 1) * 2048 // MODC) for i in range(MODC)]
    G_modv = {k: g_wmod(2048 + (k - 2) * 768, min(2048 + (k - 1) * 768, 6144)) for k in range(2, 8)}
    G_wq0 = [g_wq(a, b) for a, b in WQ0]
    G_wq = [None] + [g_wq(8 * g, 8 * g + 8) for g in range(1, HKV)]
    G_k = [g_k(g) for g in range(HKV)]
    G_v = [g_v(g) for g in range(HKV)]
    G_wo = [g_wo(g) for g in range(HKV)]
    G_ffn = Group(lambda s: [copy(wg_hbm, wg_buf, s), copy(wu_hbm, wu_buf, s),
                             copy(wd_hbm, wd_buf.at[:, pl.ds(0, D)], s)])
    s_out = new_sem()
    s_fin = new_sem()
    assert nsem[0] <= NSEM

    def cp_out(e):
        r0 = _mult(e * TQ, TQ)
        return copy(out_buf.at[pl.ds(r0, TQ)], out_hbm.at[pl.ds(r0, TQ)], s_out)

    first_order = [G_c, G_x0] + G_mod0 + [G_wq0[0], G_wq0[1], G_k[0], G_v[0]] + G_wq0[2:] + [G_x1, G_wr]
    first_order += [G_wo[0], G_xa, G_wq[1], G_k[1], G_v[1], G_xb, G_modv[2], G_wo[1], G_modv[3],
                    G_wq[2], G_k[2], G_v[2], G_modv[4], G_wo[2]]
    later_order = [G_modv[5], G_wq[3], G_k[3], G_v[3], G_modv[6], G_wo[3], G_modv[7], G_xc, G_ffn]
    for grp in first_order:
        grp.start()

    def modrow(i, nrows):
        return jnp.concatenate([mod_buf[i]] * (nrows // 8), axis=0)

    def normalize(xv):
        return _ln(xv.astype(f32))

    def store_h(hn, slot, hr0, nrows):
        h = (hn * modrow(1, nrows) + modrow(0, nrows)).astype(bf16)
        for c in range(NDT):
            h_buf[slot, c, pl.ds(hr0, nrows), :] = h[:, c * 128:(c + 1) * 128]

    def load_h(slot):
        return jnp.concatenate([h_buf[slot, c] for c in range(NDT)], axis=1)

    def qproj(t, hv):
        return (_dot(hv, wq_buf[t]) * (SCALE * LOG2E)).astype(bf16)

    def qk(g, qh):
        return jax.lax.dot_general(qh, k_buf[g], NT, preferred_element_type=f32)

    def softmax(s):
        m = jnp.max(s, axis=-1, keepdims=True)
        p = jnp.exp2(s - m)
        l = jnp.sum(p, axis=-1, keepdims=True)
        r = pl.reciprocal(l, approx=True)
        r = r * (2.0 - l * r)
        return p.astype(bf16), r

    def pv(g, p, r):
        return (_dot(p, v_buf[g]) * r).astype(bf16)

    def load_o(slot, r0=0, nrows=TM):
        return jnp.concatenate([o_buf[slot, j, pl.ds(r0, nrows), :] for j in range(REP)], axis=1)

    def epilogue(r0, att, xv):
        x1 = (xv.astype(f32) + modrow(2, CH) * att).astype(bf16)
        x_buf[pl.ds(r0, CH), :] = x1
        x1f = x1.astype(f32)
        h2b = (_ln(x1f) * modrow(4, CH) + modrow(3, CH)).astype(bf16)
        h2_buf[pl.ds(r0, CH), :] = h2b
        h2 = h2b.astype(f32)
        wr = jnp.concatenate([wrf_buf[...]] * (CH // 8), axis=0)
        r = jnp.sum(h2 * wr, axis=-1, keepdims=True)
        out_buf[pl.ds(r0, CH), :] = (x1f + modrow(5, CH) * (h2 + h2 * 0.0)).astype(bf16)
        return r

    def track(r0, r):
        rid = r0 + jax.lax.broadcasted_iota(i32, (CH, 1), 0)
        bv = best_v[...]
        upd = r > bv
        best_i[...] = jnp.where(upd, rid, best_i[...])
        best_v[...] = jnp.where(upd, r, bv)

    def mod_tiles(sc8, n0, n1):
        for n in range(n0, n1):
            d = _dot(sc8, wmod_buf[:, n * 128:(n + 1) * 128]).astype(bf16).astype(f32)
            if n // 8 in (1, 4):
                d = 1.0 + d
            mod_buf[n // 8, :, (n % 8) * 128:(n % 8 + 1) * 128] = d

    att_buf[...] = jnp.zeros(att_buf.shape, f32)
    mod_buf[...] = jnp.zeros(mod_buf.shape, f32)
    best_v[...] = jnp.full(best_v.shape, -jnp.inf, f32)
    best_i[...] = jnp.zeros(best_i.shape, i32)

    G_c.wait()
    cf = c_ref[...].astype(f32)
    sc8 = jnp.broadcast_to((cf * jax.nn.sigmoid(cf)).astype(bf16), (8, D))
    scf = sc8[0:1].astype(f32)
    for c_ in range(NDT):
        scol_buf[c_ * 128:(c_ + 1) * 128, :] = jnp.broadcast_to(scf[:, c_ * 128:(c_ + 1) * 128], (128, 128)).T
    G_x0.wait()
    hn0 = normalize(x_buf[pl.ds(0, TM), :])
    for i in range(MODC):
        G_mod0[i].wait()
        mod_tiles(sc8, i * 16 // MODC, (i + 1) * 16 // MODC)
    store_h(hn0, 0, 0, TM)

    def item(i, first, steady=False):
        par = i & 1
        g = _shr(i, 1) & 3
        pair = _shr(i, 3)
        hslot = (pair & 1) * 2 + par
        ip = i - 1
        gp = _shr(ip, 1) & 3
        aslot = (_shr(ip, 3) & 1) * 2 + (ip & 1)
        if not first:
            u_ln = ip & 7
            pn = _shr(ip, 3) + 1
            lr0 = _mult(jnp.minimum(pn * 8 + u_ln, NQ - 1) * TQ, TQ)
            lslot = (pn & 1) * 2 + _shr(u_ln, 2)
            lh0 = (u_ln & 3) * TQ
            e = i - 8
            er0 = _mult(e * TQ, TQ)
            eslot = _shr(e, 2) & 3
            ea0 = _mult((e & 3) * TQ, TQ)

        if not first and not steady:
            for k_, grps in ((1, [G_wo[0], G_xa, G_wr]), (2, [G_wq[1], G_k[1], G_v[1], G_xb]), (3, [G_wo[1]]),
                             (4, [G_wq[2], G_k[2], G_v[2]]), (5, [G_wo[2]]), (6, [G_wq[3], G_k[3], G_v[3]]),
                             (7, [G_wo[3]])):
                @pl.when(i == k_)
                def _():
                    for grp in grps:
                        grp.wait()
                    if k_ == 1:
                        wrf_buf[...] = jnp.broadcast_to(wr_ref[...].astype(f32).reshape(1, D), (8, D))
                    if k_ >= 2:
                        G_modv[k_].wait()

        hv = load_h(hslot)
        if not first:
            og = load_o(1 - par)
            xl = x_buf[pl.ds(lr0, TQ), :]
            if steady:
                xe = x_buf[pl.ds(er0, TQ), :]
                ae = att_buf[eslot, pl.ds(ea0, TQ), :]

        def do_ln(u):
            store_h(normalize(xl[u * CH:(u + 1) * CH]), lslot, _mult(lh0 + u * CH, CH), CH)

        def do_epi(u):
            r0 = _mult(er0 + u * CH, CH)
            track(r0, epilogue(r0, ae[u * CH:(u + 1) * CH], xe[u * CH:(u + 1) * CH]))

        early = not first and not steady
        if early:
            mv_n = [16 + (i - 2) * 6 + u for u in range(6)]
            mv_valid = [jnp.logical_and(i >= 2, n_ < 48) for n_ in mv_n]
            mv_src = [pl.multiple_of(jnp.where(v_, n_, 0) * 128, 128) for v_, n_ in zip(mv_valid, mv_n)]
            mv_acc = [None] * 6

        def do_modv(kk):
            col = scol_buf[kk * 128:(kk + 1) * 128, :]
            for r_ in range(0, 128, 8):
                cr = col[r_:r_ + 8]
                for u in range(6):
                    p_ = wmod_buf[kk * 128 + r_:kk * 128 + r_ + 8, pl.ds(mv_src[u], 128)].astype(f32) * cr
                    mv_acc[u] = p_ if mv_acc[u] is None else mv_acc[u] + p_

        def fin_modv():
            for u in range(6):
                d = jnp.sum(mv_acc[u], axis=0, keepdims=True).astype(bf16).astype(f32)
                n_ = mv_n[u]
                is_scale = jnp.logical_and(n_ >= 32, n_ < 40)
                d = d + jnp.where(is_scale, 1.0, 0.0)
                row = jnp.where(mv_valid[u], _shr(n_, 3), 6)
                mod_buf[row, :, pl.ds(pl.multiple_of((n_ & 7) * 128, 128), 128)] = jnp.broadcast_to(d, (8, 128))

        def qp(j):
            if first:
                for grp, (a, _) in zip(G_wq0, WQ0):
                    if a == j:
                        grp.wait()
            return qproj(g * REP + j, hv)

        qs = {0: qp(0), 1: qp(1)}
        if first:
            G_k[0].wait()
        ss = {0: qk(g, qs.pop(0))}
        for j in range(REP):
            if j + 1 < REP:
                ss[j + 1] = qk(g, qs.pop(j + 1))
            if not first:
                if j < NCH:
                    do_ln(j)
                elif steady:
                    do_epi(j - NCH)
                if early:
                    do_modv(j)
                    if j == REP - 1:
                        fin_modv()
            else:
                if j == 1:
                    for grp in later_order:
                        grp.start()
                if j == 4:
                    G_x1.wait()
                if j >= 4:
                    r0 = (j - 4) * TQ
                    store_h(normalize(x_buf[pl.ds(TM + r0, TQ), :]), 1, r0, TQ)
            if j + 2 < REP:
                qs[j + 2] = qp(j + 2)
            if not first:
                c = _dot(og, wo_buf[gp, j])
                old = att_buf[aslot, :, j * 128:(j + 1) * 128]
                att_buf[aslot, :, j * 128:(j + 1) * 128] = jnp.where(gp == 0, 0.0, old) + c
            p, r = softmax(ss.pop(j))
            if first and j == 0:
                G_v[0].wait()
            o_buf[par, j] = pv(g, p, r)
        if steady:
            cp_out(e).start()

    item(0, True)

    def early_body(i, carry):
        item(i, False)
        return carry

    def steady_body(i, carry):
        item(i, False, True)
        return carry

    jax.lax.fori_loop(1, 8, early_body, 0)
    G_xc.wait()
    jax.lax.fori_loop(8, NITEMS, steady_body, 0)

    def chunk(e, u, slot):
        r0 = e * TQ + u * CH
        r = epilogue(r0, att_buf[slot, pl.ds((e % 4) * TQ + u * CH, CH), :], x_buf[pl.ds(r0, CH), :])
        track(r0, r)
        if u == NCH - 1:
            cp_out(e).start()

    pending = [(e, u, 2) for e in range(NQ - 8, NQ - 4) for u in range(NCH)]
    for w in range(4):
        og = load_o((NITEMS - 1) % 2, w * TQ, TQ)
        for n in range(NDT):
            att_buf[3, pl.ds(w * TQ, TQ), n * 128:(n + 1) * 128] += _dot(og, wo_buf[3, n])
            if pending:
                chunk(*pending.pop(0))
        pending += [(NQ - 4 + w, u, 3) for u in range(NCH)]
    for c_ in pending:
        chunk(*c_)

    bv = best_v[...]
    mxv = jnp.max(bv, axis=0, keepdims=True)
    idxv = jnp.min(jnp.where(bv == mxv, best_i[...], S - 1), axis=0, keepdims=True)
    idx = jnp.clip(idxv[0, 0], 0, S - 1)
    base = pl.multiple_of(_shr(idx, 4) * 16, 16)
    x1f = x_buf[pl.ds(base, 16), :].astype(f32)
    h2b = h2_buf[pl.ds(base, 16), :]
    h2 = h2b.astype(f32)
    G_ffn.wait()
    acts = []
    for n in range(NFT):
        g_ = _dot(h2b, wg_buf[:, n * 128:(n + 1) * 128])
        u_ = _dot(h2b, wu_buf[:, n * 128:(n + 1) * 128])
        acts.append((g_ * jax.nn.sigmoid(g_) * u_).astype(bf16))
    a_ = jnp.concatenate(acts, axis=1)
    y = jnp.concatenate([_dot(a_, wd_buf[:, n * 128:(n + 1) * 128]) for n in range(NDT)], axis=1)
    y = y * jax.nn.sigmoid(mxv)
    rid = base + jax.lax.broadcasted_iota(i32, (16, 1), 0)
    upd = jnp.where(rid == idx, y, h2 * 0.0)
    copy(out_buf, out_hbm, s_out).wait()
    out_buf[pl.ds(base, 16), :] = (x1f + modrow(5, 16) * (h2 + upd)).astype(bf16)
    fin = copy(out_buf.at[pl.ds(base, 16)], out_hbm.at[pl.ds(base, 16)], s_fin)
    fin.start()
    fin.wait()


_SCRATCH = [
    pltpu.VMEM((S, D), bf16),
    pltpu.VMEM((HKV, W, DH), bf16),
    pltpu.VMEM((HKV, W, DH), bf16),
    pltpu.VMEM((HQ, D, 128), bf16),
    pltpu.VMEM((HKV, NDT, 1024, 128), bf16),
    pltpu.VMEM((D, F), bf16),
    pltpu.VMEM((D, F), bf16),
    pltpu.VMEM((F, D + PADW), bf16),
    pltpu.VMEM((D, 6 * D + PADW), bf16),
    pltpu.VMEM((7, 8, D), f32),
    pltpu.VMEM((4, NDT, TM, 128), bf16),
    pltpu.VMEM((2, REP, TM, 128), bf16),
    pltpu.VMEM((4, TM, D), f32),
    pltpu.VMEM((S, D), bf16),
    pltpu.VMEM((S, D), bf16),
    pltpu.VMEM((D, 128), f32),
    pltpu.VMEM((CH, 1), f32),
    pltpu.VMEM((CH, 1), i32),
    pltpu.VMEM((1, D), bf16),
    pltpu.VMEM((D,), bf16),
    pltpu.VMEM((8, D), f32),
    pltpu.SemaphoreType.DMA((NSEM,)),
]


@jax.jit
def pallas_adaLN_cond__sliding_block_cached__moe_arch_mod__prompt_kernel(
    A_x: jax.Array,
    A_k_cache: jax.Array,
    A_v_cache: jax.Array,
    A_wq: jax.Array,
    A_wo: jax.Array,
    B_x: jax.Array,
    B_w_r: jax.Array,
    B_w_gate: jax.Array,
    B_w_up: jax.Array,
    B_w_down: jax.Array,
    c: jax.Array,
    w_mod: jax.Array,
):
    del B_x
    hbm = pl.BlockSpec(memory_space=pl.ANY)
    out = pl.pallas_call(
        _kernel,
        out_shape=jax.ShapeDtypeStruct((S, D), bf16),
        in_specs=[hbm] * 11,
        out_specs=hbm,
        scratch_shapes=_SCRATCH,
        compiler_params=pltpu.CompilerParams(vmem_limit_bytes=126 * 1024 * 1024),
    )(A_x.reshape(S, D), A_k_cache.reshape(HKV, SK, DH), A_v_cache.reshape(HKV, SK, DH), A_wq, A_wo,
      B_w_r, B_w_gate, B_w_up, B_w_down, c, w_mod)
    return out.reshape(1, S, D)
```

```python
import jax
import jax.numpy as jnp
import jax.experimental.pallas as pl
import jax.experimental.pallas.tpu as pltpu

S, D, HQ, HKV, DH, SK, W, F = 2048, 1024, 32, 4, 128, 2048, 512, 3584
REP = HQ // HKV
LOG2E = 1.4426950408889634
SCALE = DH ** -0.5
EPS = 1e-5
bf16 = jnp.bfloat16
f32 = jnp.float32
i32 = jnp.int32
NT = (((1,), (1,)), ((), ()))

TM = 256
NB = S // TM
NDT = D // 128
NFT = F // 128
TQ = TM // 4
NQ = S // TQ
NITEMS = NB * HKV
CH = 16
NCH = TQ // CH
MODC = 4
PADW = 128
WQ0 = ((0, 1), (1, 2), (2, 4), (4, 8))
GW = REP * DH
NSEM = 39


def _ln(xf):
    m = jnp.mean(xf, axis=-1, keepdims=True)
    xc = xf - m
    v = jnp.mean(xc * xc, axis=-1, keepdims=True)
    return xc * jax.lax.rsqrt(v + EPS)


def _dot(a, b):
    return jnp.dot(a, b, preferred_element_type=f32)


def _shr(x, n):
    return x >> n if isinstance(x, int) else jax.lax.shift_right_logical(x, n)


def _mult(x, n):
    return x if isinstance(x, int) else pl.multiple_of(x, n)


def _kernel(x_hbm, k_hbm, v_hbm, wq_hbm, wo_hbm, wr_hbm, wg_hbm, wu_hbm, wd_hbm, c_hbm, wmod_hbm,
            out_hbm,
            x_buf, k_buf, v_buf, wq_buf, wo_buf, wg_buf, wu_buf, wd_buf, wmod_buf, mod_buf,
            h_buf, o_buf, att_buf, out_buf, h2_buf, scol_buf, best_v, best_i, c_ref, wr_ref, wrf_buf, sems):
    nsem = [0]

    def new_sem():
        nsem[0] += 1
        return nsem[0] - 1

    def copy(src, dst, sem):
        return pltpu.make_async_copy(src, dst, sems.at[sem])

    class Group:
        def __init__(self, fn):
            self.cps = fn(new_sem())

        def start(self):
            for c_ in self.cps:
                c_.start()

        def wait(self):
            for c_ in self.cps:
                c_.wait()

    def g_x(r0, r1):
        return Group(lambda s: [copy(x_hbm.at[pl.ds(r0, r1 - r0)], x_buf.at[pl.ds(r0, r1 - r0)], s)])

    def g_wq(t0, t1):
        return Group(lambda s: [copy(wq_hbm.at[:, pl.ds(t0 * DH, (t1 - t0) * DH)],
                                     wq_buf.at[t0 // REP, :, pl.ds((t0 % REP) * DH, (t1 - t0) * DH)], s)])

    def g_wo(g):
        return Group(lambda s: [copy(wo_hbm.at[pl.ds(g * GW, GW), :], wo_buf.at[g, :, pl.ds(0, D)], s)])

    def g_k(g):
        return Group(lambda s: [copy(k_hbm.at[g, pl.ds(SK - W, W), :], k_buf.at[g], s)])

    def g_v(g):
        return Group(lambda s: [copy(v_hbm.at[g, pl.ds(SK - W, W), :], v_buf.at[g], s)])

    def g_wmod(c0, c1):
        return Group(lambda s: [copy(wmod_hbm.at[:, pl.ds(c0, c1 - c0)], wmod_buf.at[:, pl.ds(c0, c1 - c0)], s)])

    G_c = Group(lambda s: [copy(c_hbm, c_ref, s)])
    G_wr = Group(lambda s: [copy(wr_hbm, wr_ref, s)])
    G_x0, G_x1 = g_x(0, TM), g_x(TM, 2 * TM)
    G_xa, G_xb, G_xc = g_x(2 * TM, 2 * TM + TQ), g_x(2 * TM + TQ, 4 * TM), g_x(4 * TM, S)
    G_mod0 = [g_wmod(i * 2048 // MODC, (i + 1) * 2048 // MODC) for i in range(MODC)]
    G_modv = {k: g_wmod(2048 + (k - 2) * 768, min(2048 + (k - 1) * 768, 6144)) for k in range(2, 8)}
    G_wq0 = [g_wq(a, b) for a, b in WQ0]
    G_wq = [None] + [g_wq(8 * g, 8 * g + 8) for g in range(1, HKV)]
    G_k = [g_k(g) for g in range(HKV)]
    G_v = [g_v(g) for g in range(HKV)]
    G_wo = [g_wo(g) for g in range(HKV)]
    G_ffn = Group(lambda s: [copy(wg_hbm, wg_buf, s), copy(wu_hbm, wu_buf, s),
                             copy(wd_hbm, wd_buf.at[:, pl.ds(0, D)], s)])
    s_out = new_sem()
    s_fin = new_sem()
    assert nsem[0] <= NSEM

    def cp_out(e):
        r0 = _mult(e * TQ, TQ)
        return copy(out_buf.at[pl.ds(r0, TQ)], out_hbm.at[pl.ds(r0, TQ)], s_out)

    for grp in ([G_c, G_x0] + G_mod0 + [G_wq0[0], G_wq0[1], G_k[0], G_v[0]] + G_wq0[2:] + [G_x1, G_wr,
                G_wo[0], G_xa, G_wq[1], G_k[1], G_v[1], G_xb, G_modv[2], G_wo[1], G_modv[3],
                G_wq[2], G_k[2], G_v[2], G_modv[4], G_wo[2], G_modv[5],
                G_wq[3], G_k[3], G_v[3], G_modv[6], G_wo[3], G_modv[7], G_xc, G_ffn]):
        grp.start()

    def modrow(i, nrows):
        return jnp.concatenate([mod_buf[i]] * (nrows // 8), axis=0)

    def normalize(xv):
        return _ln(xv.astype(f32))

    def store_h(hn, slot, hr0, nrows):
        h = (hn * modrow(1, nrows) + modrow(0, nrows)).astype(bf16)
        for c in range(NDT):
            h_buf[slot, c, pl.ds(hr0, nrows), :] = h[:, c * 128:(c + 1) * 128]

    def load_h(slot):
        return jnp.concatenate([h_buf[slot, c] for c in range(NDT)], axis=1)

    def qproj(g, j, hv):
        return (_dot(hv, wq_buf[g, :, j * DH:(j + 1) * DH]) * (SCALE * LOG2E)).astype(bf16)

    def qk(g, qh):
        return jax.lax.dot_general(qh, k_buf[g], NT, preferred_element_type=f32)

    def softmax(s):
        m = jnp.max(s, axis=-1, keepdims=True)
        p = jnp.exp2(s - m)
        l = jnp.sum(p, axis=-1, keepdims=True)
        r = pl.reciprocal(l, approx=True)
        r = r * (2.0 - l * r)
        return p.astype(bf16), r

    def pv(g, p, r):
        return (_dot(p, v_buf[g]) * r).astype(bf16)

    def load_o(slot, r0=0, nrows=TM):
        return jnp.concatenate([o_buf[slot, j, pl.ds(r0, nrows), :] for j in range(REP)], axis=1)

    def epilogue(r0, att, xv):
        x1 = (xv.astype(f32) + modrow(2, CH) * att).astype(bf16)
        x_buf[pl.ds(r0, CH), :] = x1
        x1f = x1.astype(f32)
        h2b = (_ln(x1f) * modrow(4, CH) + modrow(3, CH)).astype(bf16)
        h2_buf[pl.ds(r0, CH), :] = h2b
        h2 = h2b.astype(f32)
        wr = jnp.concatenate([wrf_buf[...]] * (CH // 8), axis=0)
        r = jnp.sum(h2 * wr, axis=-1, keepdims=True)
        out_buf[pl.ds(r0, CH), :] = (x1f + modrow(5, CH) * (h2 + h2 * 0.0)).astype(bf16)
        return r

    def track(r0, r):
        rid = r0 + jax.lax.broadcasted_iota(i32, (CH, 1), 0)
        bv = best_v[...]
        upd = r > bv
        best_i[...] = jnp.where(upd, rid, best_i[...])
        best_v[...] = jnp.where(upd, r, bv)

    def mod_tiles(sc8, n0, n1):
        for n in range(n0, n1):
            d = _dot(sc8, wmod_buf[:, n * 128:(n + 1) * 128]).astype(bf16).astype(f32)
            if n // 8 in (1, 4):
                d = 1.0 + d
            mod_buf[n // 8, :, (n % 8) * 128:(n % 8 + 1) * 128] = d

    att_buf[...] = jnp.zeros(att_buf.shape, f32)
    mod_buf[...] = jnp.zeros(mod_buf.shape, f32)
    best_v[...] = jnp.full(best_v.shape, -jnp.inf, f32)
    best_i[...] = jnp.zeros(best_i.shape, i32)

    G_c.wait()
    cf = c_ref[...].astype(f32)
    sc8 = jnp.broadcast_to((cf * jax.nn.sigmoid(cf)).astype(bf16), (8, D))
    scf = sc8[0:1].astype(f32)
    for c_ in range(NDT):
        scol_buf[c_ * 128:(c_ + 1) * 128, :] = jnp.broadcast_to(scf[:, c_ * 128:(c_ + 1) * 128], (128, 128)).T
    G_x0.wait()
    hn0 = normalize(x_buf[pl.ds(0, TM), :])
    for i in range(MODC):
        G_mod0[i].wait()
        mod_tiles(sc8, i * 16 // MODC, (i + 1) * 16 // MODC)
    store_h(hn0, 0, 0, TM)

    def item(i, first, steady=False):
        par = i & 1
        g = _shr(i, 1) & 3
        pair = _shr(i, 3)
        hslot = (pair & 1) * 2 + par
        ip = i - 1
        gp = _shr(ip, 1) & 3
        aslot = (_shr(ip, 3) & 1) * 2 + (ip & 1)
        if not first:
            u_ln = ip & 7
            pn = _shr(ip, 3) + 1
            lr0 = _mult(jnp.minimum(pn * 8 + u_ln, NQ - 1) * TQ, TQ)
            lslot = (pn & 1) * 2 + _shr(u_ln, 2)
            lh0 = (u_ln & 3) * TQ
            e = i - 8
            er0 = _mult(e * TQ, TQ)
            eslot = _shr(e, 2) & 3
            ea0 = _mult((e & 3) * TQ, TQ)

        if not first and not steady:
            for k_, grps in ((1, [G_wo[0], G_xa, G_wr]), (2, [G_wq[1], G_k[1], G_v[1], G_xb]), (3, [G_wo[1]]),
                             (4, [G_wq[2], G_k[2], G_v[2]]), (5, [G_wo[2]]), (6, [G_wq[3], G_k[3], G_v[3]]),
                             (7, [G_wo[3]])):
                @pl.when(i == k_)
                def _():
                    for grp in grps:
                        grp.wait()
                    if k_ == 1:
                        wrf_buf[...] = jnp.broadcast_to(wr_ref[...].astype(f32).reshape(1, D), (8, D))
                    if k_ >= 2:
                        G_modv[k_].wait()

        hv = load_h(hslot)
        if not first:
            og = load_o(1 - par)
            xl = x_buf[pl.ds(lr0, TQ), :]
            if steady:
                xe = x_buf[pl.ds(er0, TQ), :]
                ae = att_buf[eslot, pl.ds(ea0, TQ), :]

        def do_ln(u):
            store_h(normalize(xl[u * CH:(u + 1) * CH]), lslot, _mult(lh0 + u * CH, CH), CH)

        def do_epi(u):
            r0 = _mult(er0 + u * CH, CH)
            track(r0, epilogue(r0, ae[u * CH:(u + 1) * CH], xe[u * CH:(u + 1) * CH]))

        early = not first and not steady
        if early:
            mv_n = [16 + (i - 2) * 6 + u for u in range(6)]
            mv_valid = [jnp.logical_and(i >= 2, n_ < 48) for n_ in mv_n]
            mv_src = [pl.multiple_of(jnp.where(v_, n_, 0) * 128, 128) for v_, n_ in zip(mv_valid, mv_n)]
            mv_acc = [None] * 6

        def do_modv(kk):
            col = scol_buf[kk * 128:(kk + 1) * 128, :]
            for r_ in range(0, 128, 8):
                cr = col[r_:r_ + 8]
                for u in range(6):
                    p_ = wmod_buf[kk * 128 + r_:kk * 128 + r_ + 8, pl.ds(mv_src[u], 128)].astype(f32) * cr
                    mv_acc[u] = p_ if mv_acc[u] is None else mv_acc[u] + p_

        def fin_modv():
            for u in range(6):
                d = jnp.sum(mv_acc[u], axis=0, keepdims=True).astype(bf16).astype(f32)
                n_ = mv_n[u]
                is_scale = jnp.logical_and(n_ >= 32, n_ < 40)
                d = d + jnp.where(is_scale, 1.0, 0.0)
                row = jnp.where(mv_valid[u], _shr(n_, 3), 6)
                mod_buf[row, :, pl.ds(pl.multiple_of((n_ & 7) * 128, 128), 128)] = jnp.broadcast_to(d, (8, 128))

        def qp(j):
            if first:
                for grp, (a, _) in zip(G_wq0, WQ0):
                    if a == j:
                        grp.wait()
            return qproj(g, j, hv)

        qs = {0: qp(0), 1: qp(1)}
        if first:
            G_k[0].wait()
        ss = {0: qk(g, qs.pop(0))}
        for j in range(REP):
            if j + 1 < REP:
                ss[j + 1] = qk(g, qs.pop(j + 1))
            if not first:
                if j < NCH:
                    do_ln(j)
                elif steady:
                    do_epi(j - NCH)
                if early:
                    do_modv(j)
                    if j == REP - 1:
                        fin_modv()
            else:
                if j == 4:
                    G_x1.wait()
                if j >= 4:
                    r0 = (j - 4) * TQ
                    store_h(normalize(x_buf[pl.ds(TM + r0, TQ), :]), 1, r0, TQ)
            if j + 2 < REP:
                qs[j + 2] = qp(j + 2)
            if not first:
                c = _dot(og, wo_buf[gp, :, j * 128:(j + 1) * 128])
                old = att_buf[aslot, :, j * 128:(j + 1) * 128]
                att_buf[aslot, :, j * 128:(j + 1) * 128] = jnp.where(gp == 0, 0.0, old) + c
            p, r = softmax(ss.pop(j))
            if first and j == 0:
                G_v[0].wait()
            o_buf[par, j] = pv(g, p, r)
        if steady:
            cp_out(e).start()

    item(0, True)

    def early_body(i, carry):
        item(i, False)
        return carry

    def steady_body(i, carry):
        item(i, False, True)
        return carry

    jax.lax.fori_loop(1, 8, early_body, 0)
    G_xc.wait()
    jax.lax.fori_loop(8, NITEMS, steady_body, 0)

    def chunk(e, u, slot):
        r0 = e * TQ + u * CH
        r = epilogue(r0, att_buf[slot, pl.ds((e % 4) * TQ + u * CH, CH), :], x_buf[pl.ds(r0, CH), :])
        track(r0, r)
        if u == NCH - 1:
            cp_out(e).start()

    pending = [(e, u, 2) for e in range(NQ - 8, NQ - 4) for u in range(NCH)]
    for w in range(4):
        og = load_o((NITEMS - 1) % 2, w * TQ, TQ)
        for n in range(NDT):
            att_buf[3, pl.ds(w * TQ, TQ), n * 128:(n + 1) * 128] += _dot(og, wo_buf[3, :, n * 128:(n + 1) * 128])
            if pending:
                chunk(*pending.pop(0))
        pending += [(NQ - 4 + w, u, 3) for u in range(NCH)]
    for c_ in pending:
        chunk(*c_)

    bv = best_v[...]
    mxv = jnp.max(bv, axis=0, keepdims=True)
    idxv = jnp.min(jnp.where(bv == mxv, best_i[...], S - 1), axis=0, keepdims=True)
    idx = jnp.clip(idxv[0, 0], 0, S - 1)
    base = pl.multiple_of(_shr(idx, 4) * 16, 16)
    x1f = x_buf[pl.ds(base, 16), :].astype(f32)
    h2b = h2_buf[pl.ds(base, 16), :]
    h2 = h2b.astype(f32)
    G_ffn.wait()
    acts = []
    for n in range(NFT):
        g_ = _dot(h2b, wg_buf[:, n * 128:(n + 1) * 128])
        u_ = _dot(h2b, wu_buf[:, n * 128:(n + 1) * 128])
        acts.append((g_ * jax.nn.sigmoid(g_) * u_).astype(bf16))
    a_ = jnp.concatenate(acts, axis=1)
    y = jnp.concatenate([_dot(a_, wd_buf[:, n * 128:(n + 1) * 128]) for n in range(NDT)], axis=1)
    y = y * jax.nn.sigmoid(mxv)
    rid = base + jax.lax.broadcasted_iota(i32, (16, 1), 0)
    upd = jnp.where(rid == idx, y, h2 * 0.0)
    copy(out_buf, out_hbm, s_out).wait()
    out_buf[pl.ds(base, 16), :] = (x1f + modrow(5, 16) * (h2 + upd)).astype(bf16)
    fin = copy(out_buf.at[pl.ds(base, 16)], out_hbm.at[pl.ds(base, 16)], s_fin)
    fin.start()
    fin.wait()


_SCRATCH = [
    pltpu.VMEM((S, D), bf16),
    pltpu.VMEM((HKV, W, DH), bf16),
    pltpu.VMEM((HKV, W, DH), bf16),
    pltpu.VMEM((HKV, D, GW + PADW), bf16),
    pltpu.VMEM((HKV, GW, D + PADW), bf16),
    pltpu.VMEM((D, F), bf16),
    pltpu.VMEM((D, F), bf16),
    pltpu.VMEM((F, D + PADW), bf16),
    pltpu.VMEM((D, 6 * D + PADW), bf16),
    pltpu.VMEM((7, 8, D), f32),
    pltpu.VMEM((4, NDT, TM, 128), bf16),
    pltpu.VMEM((2, REP, TM, 128), bf16),
    pltpu.VMEM((4, TM, D), f32),
    pltpu.VMEM((S, D), bf16),
    pltpu.VMEM((S, D), bf16),
    pltpu.VMEM((D, 128), f32),
    pltpu.VMEM((CH, 1), f32),
    pltpu.VMEM((CH, 1), i32),
    pltpu.VMEM((1, D), bf16),
    pltpu.VMEM((D,), bf16),
    pltpu.VMEM((8, D), f32),
    pltpu.SemaphoreType.DMA((NSEM,)),
]


@jax.jit
def pallas_adaLN_cond__sliding_block_cached__moe_arch_mod__prompt_kernel(
    A_x: jax.Array,
    A_k_cache: jax.Array,
    A_v_cache: jax.Array,
    A_wq: jax.Array,
    A_wo: jax.Array,
    B_x: jax.Array,
    B_w_r: jax.Array,
    B_w_gate: jax.Array,
    B_w_up: jax.Array,
    B_w_down: jax.Array,
    c: jax.Array,
    w_mod: jax.Array,
):
    del B_x
    hbm = pl.BlockSpec(memory_space=pl.ANY)
    out = pl.pallas_call(
        _kernel,
        out_shape=jax.ShapeDtypeStruct((S, D), bf16),
        in_specs=[hbm] * 11,
        out_specs=hbm,
        scratch_shapes=_SCRATCH,
        compiler_params=pltpu.CompilerParams(vmem_limit_bytes=126 * 1024 * 1024),
    )(A_x.reshape(S, D), A_k_cache.reshape(HKV, SK, DH), A_v_cache.reshape(HKV, SK, DH), A_wq, A_wo,
      B_w_r, B_w_gate, B_w_up, B_w_down, c, w_mod)
    return out.reshape(1, S, D)
```
